```python
import os as _os
_os.environ.setdefault("JAX_PLATFORMS", "cpu")
import jax
import jax.numpy as jnp

def _softmax(x, axis=-1):
    return jax.nn.softmax(x, axis=axis)
def _gelu(x):
    return jax.nn.gelu(x, approximate=True)
def _silu(x):
    return jax.nn.silu(x)
def _sigmoid(x):
    return jax.nn.sigmoid(x)
def _layernorm(x, axis=-1, eps=1e-5):
    m = jnp.mean(x, axis=axis, keepdims=True)
    v = jnp.var(x, axis=axis, keepdims=True)
    return (x - m) / jnp.sqrt(v + eps)
def _scatter_add(tgt, idx, src, axis=0):
    return tgt.at[idx].add(src)
def _segment_sum(src, seg, n):
    return jax.ops.segment_sum(src, seg, n)
class _Rng:
    def __init__(self, key):
        self._k = key
    def _next(self):
        self._k, sub = jax.random.split(self._k)
        return sub
    def normal(self, shape):
        return jax.random.normal(self._next(), shape, dtype=jnp.bfloat16)
    def randint(self, lo, hi, shape):
        return jax.random.randint(self._next(), shape, lo, hi, dtype=jnp.int32)
    def uniform(self, shape, lo=0.0, hi=1.0):
        return jax.random.uniform(self._next(), shape, jnp.bfloat16, lo, hi)
    def permutation(self, n):
        return jax.random.permutation(self._next(), n)


kernel_name = 'sequential_preLN__softmax_full_mha__dense_activation_gelu__prompt'

def setup_inputs():
    _rng = _Rng(jax.random.key(int.from_bytes(__import__("os").urandom(4), "little")))
    _w = (lambda a: (lambda t: t.astype(jnp.bfloat16) if jnp.issubdtype(t.dtype, jnp.floating) else t)(jnp.asarray(a)))
    def _A_setup():
        B, S, D = 1, 2048, 512
        return {
            "x": _w((lambda *s: _rng.normal(s) * 0.05)(B, S, D)),
            "wqkv": _w((lambda *s: _rng.normal(s) * 0.05)(D, 3 * D)),
            "wo": _w((lambda *s: _rng.normal(s) * 0.05)(D, D)),
        }
    _A_in = _A_setup()

    def _B_setup():
        B, S, D, F = 1, 2048, 512, 1792
        return {
            "x": _w((lambda *s: _rng.normal(s) * 0.05)(B, S, D)),
            "w1": _w((lambda *s: _rng.normal(s) * 0.4)(D, F) * (D ** -0.5)),
            "b1": _w((lambda *s: _rng.normal(s) * 0.4)(F) * 0.01),
            "w2": _w((lambda *s: _rng.normal(s) * 0.4)(F, D) * (F ** -0.5)),
            "b2": _w((lambda *s: _rng.normal(s) * 0.05)(D) * 0.01),
        }
    _B_in = _B_setup()

    return {
        "A_x": _A_in["x"],
        "A_wqkv": _A_in["wqkv"],
        "A_wo": _A_in["wo"],
        "B_x": _B_in["x"],
        "B_w1": _B_in["w1"],
        "B_b1": _B_in["b1"],
        "B_w2": _B_in["w2"],
        "B_b2": _B_in["b2"],
    }

def reference(A_x, A_wqkv, A_wo, B_x, B_w1, B_b1, B_w2, B_b2):
    def _A_ref(x, wqkv, wo):
        B, S, D = x.shape
        H = 32; Dh = D // H
        qkv = (lambda x, *d: x.transpose(*d))((x @ wqkv).reshape(B, S, 3, H, Dh), 2, 0, 3, 1, 4)
        q, k, v = qkv[0], qkv[1], qkv[2]
        scale = Dh ** -0.5
        scores = jnp.einsum("bhqd,bhkd->bhqk", q, k) * scale
        p = _softmax(scores, axis=-1)
        o = jnp.einsum("bhqk,bhkd->bhqd", p, v)
        return (lambda x, *d: x.transpose(*d))(o, 0, 2, 1, 3).reshape(B, S, D) @ wo

    def _B_ref(x, w1, b1, w2, b2):
        h = jnp.einsum("bsd,df->bsf", x, w1) + b1
        h = _gelu(h)
        return jnp.einsum("bsf,fd->bsd", h, w2) + b2

    x = A_x
    h = x + _A_ref(_layernorm(x, axis=-1), A_wqkv, A_wo)
    h2 = h + _B_ref(_layernorm(h, axis=-1), B_w1, B_b1, B_w2, B_b2)
    return h2
```

```python
import functools
import math

import jax
import jax.numpy as jnp
from jax import lax
from jax.experimental import pallas as pl
from jax.experimental.pallas import tpu as pltpu

f32, bf16, u32 = jnp.float32, jnp.bfloat16, jnp.uint32
H = 32
EPS = 1e-5
KNAME = "fused_block"


def _layernorm(x):
    mu = jnp.mean(x, axis=-1, keepdims=True)
    xc = x - mu
    var = jnp.mean(xc * xc, axis=-1, keepdims=True)
    return xc * lax.rsqrt(var + EPS)


def _gelu(x):
    c = math.sqrt(2.0 / math.pi)
    u = x * (c + (c * 0.044715) * (x * x))
    hx = 0.5 * x
    return hx + hx * jnp.tanh(u)


def _kernel(x_hbm, wqkv_hbm, wo_hbm, w1_hbm, b1_hbm, w2_hbm, b2_hbm, out_hbm,
            x_buf, wqkv, wo, w1, b1, w2, b2, out_buf,
            k_buf, qt_buf, vt_buf, ot_buf, s0, s1, in_sems, out_sems,
            *, S, D, F, bq, kc, bm1, sub1, bm3, sub3, fc, lag, dep, phases):
    dh = D // H
    n_grp = D // 128
    hpg = 128 // dh
    nq = S // bq
    nc = S // kc
    nb1 = S // bm1
    nb3 = S // bm3
    q_scale = dh ** -0.5 * math.log2(math.e)

    def x_copy(i):
        rows = pl.ds(i * bm1, bm1)
        return pltpu.make_async_copy(x_hbm.at[0, rows], x_buf.at[rows], in_sems.at[i])

    w_copies = [
        pltpu.make_async_copy(src, dst, in_sems.at[nb1 + n])
        for n, (src, dst) in enumerate(
            [(wqkv_hbm, wqkv), (wo_hbm, wo), (w1_hbm, w1), (w2_hbm, w2), (b1_hbm, b1), (b2_hbm, b2)])
    ]

    def out_copy(i):
        rows = pl.ds(pl.multiple_of(i * bm3, bm3), bm3)
        return pltpu.make_async_copy(out_buf.at[rows], out_hbm.at[0, rows], out_sems.at[i])

    x_copy(0).start()
    w_copies[0].start()
    for i in range(1, nb1):
        x_copy(i).start()
    for c in w_copies[1:]:
        c.start()
    w_copies[0].wait()

    def qkv_block(i, _):
        x_copy(i).wait()
        for s in range(bm1 // sub1):
            r0 = pl.multiple_of(i * bm1 + s * sub1, sub1)
            ln = _layernorm(x_buf[pl.ds(r0, sub1), :].astype(f32)).astype(bf16)
            k = jnp.dot(ln, wqkv[:, D:2 * D], preferred_element_type=f32).astype(bf16)
            k = pltpu.bitcast(k, u32)
            for g in range(n_grp):
                k_buf[g, pl.ds(pl.multiple_of(r0 // 2, sub1 // 2), sub1 // 2), :] = k[:, g * 128:(g + 1) * 128]
            q = jnp.dot(ln, wqkv[:, :D], preferred_element_type=f32) * q_scale
            qt = pltpu.bitcast(q.T.astype(bf16), u32)
            v = jnp.dot(ln, wqkv[:, 2 * D:], preferred_element_type=f32)
            vt = pltpu.bitcast(v.T.astype(bf16), u32)
            blk = r0 // 128
            for t in range(sub1 // 128):
                qt_buf[blk + t] = qt[:, t * 128:(t + 1) * 128]
                vt_buf[blk + t] = vt[:, t * 128:(t + 1) * 128]
        return None

    if 1 in phases:
        lax.fori_loop(0, nb1, qkv_block, None)
    else:
        for i in range(nb1):
            x_copy(i).wait()

    tq = bq // 128

    def load_q(qb, g, i):
        rows = pl.ds(pl.multiple_of((g * hpg + i) * (dh // 2), dh // 2), dh // 2)
        q = jnp.concatenate([qt_buf[qb * tq + t, rows, :] for t in range(tq)], axis=1)
        if i:
            q = jnp.concatenate([jnp.zeros((i * dh // 2, bq), u32), q], axis=0)
        return pltpu.bitcast(q, bf16)

    def qk_chunk(g, i, q, j, m, s_ref):
        kk = pltpu.bitcast(k_buf[g, pl.ds(j * kc // 2, kc // 2), :], bf16)[:, :(i + 1) * dh]
        s = jnp.dot(kk, q, preferred_element_type=f32)
        s_ref[pl.ds(j * kc, kc), :] = s
        for r in range(kc // 8):
            sr = s[r * 8:(r + 1) * 8]
            m = sr if m is None else jnp.maximum(m, sr)
        return m

    def pv_chunk(g, i, j, m, l, o, s_ref):
        ps = [None] * (kc // 8)
        for t in range(kc // 128):
            for r in reversed(range(t * 16, (t + 1) * 16)):
                p = jnp.exp2(s_ref[pl.ds(j * kc + r * 8, 8), :] - m)
                l = p if l is None else l + p
                ps[r] = p
        p = jnp.concatenate(ps, axis=0).astype(bf16)
        rows = pl.ds(pl.multiple_of((g * hpg + i) * (dh // 2), dh // 2), dh // 2)
        v = jnp.concatenate([vt_buf[j * (kc // 128) + t, rows, :] for t in range(kc // 128)], axis=1)
        oc = jnp.dot(pltpu.bitcast(v, bf16), p, preferred_element_type=f32)
        return l, (oc if o is None else o + oc)

    def row_max(m):
        return jnp.broadcast_to(jnp.max(m, axis=0, keepdims=True), m.shape)

    def store_o(qb, g, i, l, o):
        o = o * (1.0 / jnp.sum(l, axis=0, keepdims=True))
        rows = pl.ds(pl.multiple_of((g * hpg + i) * dh, dh), dh)
        for t in range(tq):
            ot_buf[qb * tq + t, rows, :] = o[:, t * 128:(t + 1) * 128]

    def attn_group(t, m_first):
        qb, g = t // n_grp, t % n_grp
        tn = jnp.minimum(t + 1, nq * n_grp - 1)
        qb_n, g_n = tn // n_grp, tn % n_grp
        bufs = (s0, s1)
        m_final = {0: m_first}
        hist = []
        m_run = l = o = q = None
        for n in range(hpg * nc + lag):
            if n < hpg * nc:
                i, j = divmod(n, nc)
                last = i + 1 == hpg
                if j == 0:
                    q = load_q(qb_n, g_n, 0) if last else load_q(qb, g, i + 1)
                    m_run = None
                m_run = qk_chunk(g_n if last else g, 0 if last else i + 1, q, j, m_run, bufs[(i + 1) % 2])
                hist.append(m_run)
                if j == nc - 1:
                    m_final[i + 1] = row_max(m_run)
            if n >= lag:
                i, j = divmod(n - lag, nc)
                m = m_final[i]
                d = min(n, hpg * nc - 1) - dep
                if dep and d >= 0:
                    m = jnp.maximum(m, jnp.minimum(m, hist[d]))
                if j == 0:
                    l = o = None
                l, o = pv_chunk(g, i, j, m, l, o, bufs[i % 2])
                if j == nc - 1:
                    store_o(qb, g, i, l, o)
        return m_final[hpg]

    if 2 in phases:
        q = load_q(0, 0, 0)
        m = None
        for j in range(nc):
            m = qk_chunk(0, 0, q, j, m, s0)
        lax.fori_loop(0, nq * n_grp, attn_group, row_max(m))

    for c in w_copies[1:]:
        c.wait()

    def mlp_block(i, _):
        b1v = b1[...].astype(f32).reshape(1, F)
        b2v = b2[...].astype(f32).reshape(1, D)
        ns = bm3 // sub3
        hs, lns = [], []
        for s in range(ns):
            r0 = pl.multiple_of(i * bm3 + s * sub3, sub3)
            blk = r0 // 128
            o = jnp.concatenate([ot_buf[blk + t].T for t in range(sub3 // 128)], axis=0).astype(bf16)
            h = x_buf[pl.ds(r0, sub3), :].astype(f32) + jnp.dot(o, wo[...], preferred_element_type=f32)
            hs.append(h)
            lns.append(_layernorm(h).astype(bf16))
        for s in range(ns):
            r0 = pl.multiple_of(i * bm3 + s * sub3, sub3)
            acc = hs[s] + b2v
            prev = None
            nfc = F // fc
            for c in range(nfc + 1):
                if c < nfc:
                    cols = slice(c * fc, (c + 1) * fc)
                    mid = jnp.dot(lns[s], w1[:, cols], preferred_element_type=f32) + b1v[:, cols]
                    cur = _gelu(mid).astype(bf16)
                if prev is not None:
                    acc = acc + jnp.dot(prev, w2[(c - 1) * fc:c * fc, :], preferred_element_type=f32)
                prev = cur
            out_buf[pl.ds(r0, sub3), :] = acc.astype(bf16)
        out_copy(i).start()
        return None

    if 3 in phases:
        lax.fori_loop(0, nb3, mlp_block, None)
    else:
        out_buf[...] = jnp.zeros(out_buf.shape, bf16)
        for i in range(nb3):
            out_copy(i).start()
    for i in range(nb3):
        out_copy(i).wait()


def make(variant="", bq=512, kc=128, bm1=512, sub1=128, bm3=512, sub3=256, fc=256, lag=1, dep=2,
         phases=(1, 2, 3), flags=None):
    def f(A_x, A_wqkv, A_wo, B_x, B_w1, B_b1, B_w2, B_b2):
        del B_x
        _, S, D = A_x.shape
        F = B_w1.shape[1]
        kern = functools.partial(_kernel, S=S, D=D, F=F, bq=bq, kc=kc, bm1=bm1, sub1=sub1, bm3=bm3, sub3=sub3,
                                 fc=fc, lag=lag, dep=dep, phases=tuple(phases))
        any_spec = pl.BlockSpec(memory_space=pl.ANY)
        return pl.pallas_call(
            kern,
            in_specs=[any_spec] * 7,
            out_specs=any_spec,
            out_shape=jax.ShapeDtypeStruct(A_x.shape, A_x.dtype),
            scratch_shapes=[
                pltpu.VMEM((S, D), bf16), pltpu.VMEM((D, 3 * D), bf16), pltpu.VMEM((D, D), bf16),
                pltpu.VMEM((D, F), bf16), pltpu.VMEM((F,), bf16), pltpu.VMEM((F, D), bf16), pltpu.VMEM((D,), bf16),
                pltpu.VMEM((S, D), bf16),
                pltpu.VMEM((D // 128, S // 2, 128), u32), pltpu.VMEM((S // 128, D // 2, 128), u32),
                pltpu.VMEM((S // 128, D // 2, 128), u32), pltpu.VMEM((S // 128, D, 128), f32),
                pltpu.VMEM((S, bq), f32), pltpu.VMEM((S, bq), f32),
                pltpu.SemaphoreType.DMA((S // bm1 + 6,)), pltpu.SemaphoreType.DMA((S // bm3,)),
            ],
            compiler_params=pltpu.CompilerParams(vmem_limit_bytes=100 * 2**20, flags=flags),
            name=KNAME,
        )(A_x, A_wqkv, A_wo, B_w1, B_b1, B_w2, B_b2)
    return f


@jax.jit
def pallas_sequential_preLN__softmax_full_mha__dense_activation_gelu__prompt_kernel(
    A_x, A_wqkv, A_wo, B_x, B_w1, B_b1, B_w2, B_b2,
):
    return make()(A_x, A_wqkv, A_wo, B_x, B_w1, B_b1, B_w2, B_b2)
```

```python
import functools
import math

import jax
import jax.numpy as jnp
from jax import lax
from jax.experimental import pallas as pl
from jax.experimental.pallas import tpu as pltpu

f32, bf16, u32 = jnp.float32, jnp.bfloat16, jnp.uint32
H = 32
EPS = 1e-5
KNAME = "fused_block"
L_MIN, L_MAX = 2.0 ** -40, 2.0 ** 60
F32_MAX = 3.0e38


def _layernorm(x):
    mu = jnp.mean(x, axis=-1, keepdims=True)
    xc = x - mu
    var = jnp.mean(xc * xc, axis=-1, keepdims=True)
    return xc * lax.rsqrt(var + EPS)


def _gelu(x):
    c = math.sqrt(2.0 / math.pi)
    u = x * (c + (c * 0.044715) * (x * x))
    hx = 0.5 * x
    return hx + hx * jnp.tanh(u)


def _dot(a, b):
    return jnp.dot(a, b, preferred_element_type=f32)


def _strassen_rhs(w_ref, t_ref, r, n, keep=None, after=None):
    kh, nh = w_ref.shape[0] // 2, w_ref.shape[1] // 2
    top = w_ref[pl.ds(r, n), :].astype(f32)
    bot = w_ref[pl.ds(kh + r, n), :].astype(f32)
    b11, b12, b21, b22 = top[:, :nh], top[:, nh:], bot[:, :nh], bot[:, nh:]
    if after is not None:
        rep = (n // 8, nh // 128)
        b11 = jnp.where(jnp.tile(keep, rep), b11, jnp.tile(after, rep))
        b22 = jnp.where(jnp.tile(keep, rep), b22, jnp.tile(after, rep))
    for i, t in enumerate((b11 + b22, b12 - b22, b21 - b11, b11 + b12, b21 + b22)):
        t_ref[i, pl.ds(r, n), :] = t.astype(bf16)


def _strassen_lhs(a11, a12, a21, a22):
    return [t.astype(bf16) for t in (a11 + a22, a21 + a22, a11, a22, a11 + a12, a21 - a11, a12 - a22)]


def _strassen_out(m):
    return m[0] + m[3] - m[4] + m[6], m[2] + m[4], m[1] + m[3], m[0] - m[1] + m[2] + m[5]


def _rhs_blocks(w_ref, t_ref, rows, cols):
    kh, nh = w_ref.shape[0] // 2, w_ref.shape[1] // 2
    rows2 = slice(kh + rows.start, kh + rows.stop)
    cols2 = slice(nh + cols.start, nh + cols.stop)
    return [t_ref[0, rows, cols], w_ref[rows, cols], t_ref[1, rows, cols], t_ref[2, rows, cols],
            w_ref[rows2, cols2], t_ref[3, rows, cols], t_ref[4, rows, cols]]


def _matmul(a, w_ref, t_ref):
    kh, nh = w_ref.shape[0] // 2, w_ref.shape[1] // 2
    if t_ref is None:
        r = _dot(a.astype(bf16), w_ref[...])
        return r[:, :nh], r[:, nh:]
    mh = a.shape[0] // 2
    lhs = _strassen_lhs(a[:mh, :kh], a[:mh, kh:], a[mh:, :kh], a[mh:, kh:])
    c11, c12, c21, c22 = _strassen_out(
        [_dot(x, y) for x, y in zip(lhs, _rhs_blocks(w_ref, t_ref, slice(0, kh), slice(0, nh)))])
    return jnp.concatenate([c11, c21], axis=0), jnp.concatenate([c12, c22], axis=0)


def _kernel(x_hbm, wqkv_hbm, wo_hbm, w1_hbm, b1_hbm, w2_hbm, b2_hbm, out_hbm,
            x_buf, wq, wkv, wo, w1, b1, w2, b2, out_buf, ln_buf,
            k_buf, qt_buf, vt_buf, ot_buf, kf_buf, qv_buf, kb0, kb1, kl0, kl1, tq_buf, tkv, to, t1, t2,
            x_sems, w_sems, out_sems,
            *, S, D, F, bq, kc, bma, suba, bmb, subb, bm3, sub3, fc, lag, phases, rv, kgb, heads, tie, tie_d,
            qtie, tie_off, carry_over, st_q, st_kv, st_o, st_f, xparts, prep_in_b, rvs, ncb, fill_lead, atie, after_mode, late_w, oinit, pf32, rollb):
    dh = D // H
    n_grp = D // 128
    hpg = 128 // dh
    nq = S // bq
    nc = S // kc
    tq = bq // 128
    q_scale = dh ** -0.5 * math.log2(math.e)

    xb = [0] + list(xparts)
    x_copies = [pltpu.make_async_copy(x_hbm.at[0, pl.ds(a, b - a)], x_buf.at[pl.ds(a, b - a)], x_sems.at[n])
                for n, (a, b) in enumerate(zip(xb[:-1], xb[1:]))]
    wq_copy, wkv_copy, w1_copy, w2_copy, wo_copy, b1_copy, b2_copy = [
        pltpu.make_async_copy(src, dst, w_sems.at[n])
        for n, (src, dst) in enumerate(
            [(wqkv_hbm.at[:, pl.ds(0, D)], wq), (wqkv_hbm.at[:, pl.ds(D, 2 * D)], wkv), (w1_hbm, w1), (w2_hbm, w2),
             (wo_hbm, wo), (b1_hbm, b1.at[pl.ds(0, F)]), (b2_hbm, b2.at[pl.ds(0, D)])])
    ]

    def out_copy(i):
        rows = pl.ds(pl.multiple_of(i * sub3, sub3), sub3)
        return pltpu.make_async_copy(out_buf.at[rows], out_hbm.at[0, rows], out_sems.at[i])

    late = (w1_copy, w2_copy, wo_copy, b1_copy, b2_copy)
    for c in (x_copies[0], wq_copy, *x_copies[1:], wkv_copy) + (() if late_w else late):
        c.start()

    def q_rows(r0, after):
        x = x_buf[pl.ds(r0, suba), :].astype(f32)
        if after is not None:
            x = jnp.where((after == after) | (after != after), x, after) if after_mode == 0 else jnp.where(keep_a, x, after)
        ln = _layernorm(x)
        ln_buf[pl.ds(r0, suba), :] = ln if st_kv else ln.astype(bf16)
        q0 = jnp.concatenate(_matmul(ln, wq, tq_buf if st_q else None), axis=1)
        q = q0 * q_scale
        qt = pltpu.bitcast(q.T.astype(bf16), u32)
        for t in range(suba // 128):
            for h in range(H):
                qt_buf[h, r0 // 128 + t] = qt[h * 8:(h + 1) * 8, t * 128:(t + 1) * 128]
        return q0

    def kv_block(i, _):
        fill = []
        keep = lax.broadcasted_iota(jnp.int32, (8, 128), 0) >= i // S
        for t in range(bmb // 128):
            blk = i * (bmb // 128) + t
            if rv:
                for h in range(H):
                    def stage_q(after, blk=blk, h=h):
                        qf = pltpu.bitcast(jnp.where(keep, qt_buf[h, blk], pltpu.bitcast(after, u32)), bf16).astype(f32)
                        for d in range(dh):
                            qv_buf[blk, h * dh + d] = jnp.broadcast_to(qf[d:d + 1], (8, 128))
                    fill.append(stage_q)
        if st_f and prep_in_b:
            n1, n2 = D // 2 // (S // bmb), F // 2 // (S // bmb)
            extra = [functools.partial(_strassen_rhs, w1, t1, pl.multiple_of(i * n1 + r, 16), 16, keep) for r in range(0, n1, 16)]
            if prep_in_b > 1:
                extra += [functools.partial(_strassen_rhs, w2, t2, pl.multiple_of(i * n2 + r, 32), 32, keep)
                          for r in range(0, n2, 32)]
            step = max(len(fill) // len(extra), 1)
            for n, e in enumerate(extra):
                fill.insert(n * (step + 1), e)
        n_dots = (bmb // subb) * ((7 * D // ncb) if st_kv else (2 * D // ncb))
        count = [0, 0]

        def dot(a, b):
            r = _dot(a, b)
            count[0] += 1
            first, last = count[1], min((count[0] + fill_lead) * len(fill) // n_dots, len(fill))
            for n in range(first, last):
                a = (n - first) * (r.shape[0] // 8) // (last - first) * 8
                fill[n](r[a:a + 8, :128])
            count[1] = max(last, first)
            return r

        for s in range(bmb // subb):
            r0 = pl.multiple_of(i * bmb + s * subb, subb)
            ln = ln_buf[pl.ds(r0, subb), :]
            if st_kv:
                mh, kh = subb // 2, D // 2
                lhs = _strassen_lhs(ln[:mh, :kh], ln[:mh, kh:], ln[mh:, :kh], ln[mh:, kh:])
                ks, vs = [], []
                for c in range(0, D, ncb):
                    c11, c12, c21, c22 = _strassen_out(
                        [dot(x, y) for x, y in zip(lhs, _rhs_blocks(wkv, tkv, slice(0, kh), slice(c, c + ncb)))])
                    ks.append(jnp.concatenate([c11, c21], axis=0))
                    vs.append(jnp.concatenate([c12, c22], axis=0))
                k, v = jnp.concatenate(ks, axis=1), jnp.concatenate(vs, axis=1)
            else:
                lnb = ln.astype(bf16)
                v = jnp.concatenate([dot(lnb, wkv[:, D + c:D + c + ncb]) for c in range(0, D, ncb)], axis=1)
                k = jnp.concatenate([dot(lnb, wkv[:, c:c + ncb]) for c in range(0, D, ncb)], axis=1)
            vt = pltpu.bitcast(v.T.astype(bf16), u32)
            kk = k.astype(bf16)
            ku = pltpu.bitcast(kk, u32)
            for g in range(n_grp):
                k_buf[g, pl.ds(pl.multiple_of(r0 // 2, subb // 2), subb // 2), :] = ku[:, g * 128:(g + 1) * 128]
            for t in range(subb // 128):
                blk = r0 // 128 + t
                for h in range(H):
                    vt_buf[h, blk] = vt[h * 8:(h + 1) * 8, t * 128:(t + 1) * 128]
                if rv:
                    for g in range(n_grp):
                        kf_buf[g, blk] = kk[t * kc:t * kc + rv, g * 128:(g + 1) * 128].astype(f32)
        return None

    if 1 in phases:
        waited = 0
        qs = []
        keep_a = None
        if bma < S:
            wq_copy.wait()

            def q_block(i, _):
                rows = pl.ds(pl.multiple_of(i * bma, bma), bma)
                pltpu.make_async_copy(x_hbm.at[0, rows], x_buf.at[rows], x_sems.at[i]).wait()
                for s in range(bma // suba):
                    q_rows(pl.multiple_of(i * bma + s * suba, suba), None)
                return None

            lax.fori_loop(0, S // bma, q_block, None)
        for r0 in range(0, S if bma == S else 0, suba):
            while xb[waited] < r0 + suba:
                x_copies[waited].wait()
                waited += 1
                qs = []
                if keep_a is None:
                    probe = x_buf[0:16, 0:128].astype(f32)[:8]
                    keep_a = jnp.tile(pltpu.bitcast(probe, u32) & 1 == 0, (suba // 8, D // 128))
            if r0 == 0:
                wq_copy.wait()
                if st_q:
                    for r in range(0, D // 2, 32):
                        _strassen_rhs(wq, tq_buf, r, 32)
            qs.append(q_rows(r0, qs[-atie] if atie and len(qs) >= atie else None))
        if late_w == 1:
            for c in late:
                c.start()
        wkv_copy.wait()
        if st_kv:
            for r in range(0, D // 2, 32):
                _strassen_rhs(wkv, tkv, r, 32)
        if st_f and prep_in_b:
            w1_copy.wait()
            if prep_in_b > 1:
                w2_copy.wait()
        lax.fori_loop(0, S // bmb, kv_block, None)
        if late_w == 2:
            for c in late:
                c.start()
    else:
        if late_w:
            for c in late:
                c.start()
        for c in (*x_copies, wq_copy, wkv_copy):
            c.wait()

    rv_of = [rvs[j % len(rvs)] if rvs else rv for j in range(nc)]
    kbs = (kb0, kb1)
    kls = (kl0, kl1)

    def order_of(j):
        return list(reversed(range(rv_of[j] // 16, kc // 16)))

    def store_o(qb, h, l, o, bad):
        l = jnp.sum(l, axis=0, keepdims=True)
        o = o * (1.0 / l)
        rows = pl.ds(pl.multiple_of(h * dh, dh), dh)
        for t in range(tq):
            ot_buf[qb * tq + t, rows, :] = o[:, t * 128:(t + 1) * 128]
        ok = (l >= L_MIN) & (l <= L_MAX) & (jnp.abs(o[:8]) + jnp.abs(o[8:]) <= F32_MAX)
        return jnp.where(ok, bad, 1.0)

    def stage(h, j, par, part, nparts):
        g = h // hpg
        shift = (128 - (h % hpg) * dh) % 128
        order = order_of(j)
        n = len(order)
        for a in range(part * n // nparts, (part + 1) * n // nparts):
            kls[par][a] = pltpu.roll(k_buf[g, pl.ds((j * kc + order[a] * 16) // 2, 8), :], shift, 1)
        kf = {}
        n_kb = rv_of[j] // 8 * dh
        for e in range(part * n_kb // nparts, (part + 1) * n_kb // nparts):
            r, d = divmod(e, dh)
            if rollb:
                src = pltpu.roll(kf_buf[g, j, r * 8:(r + 1) * 8, :], (shift + 128 - d) % 128, 1)
                kbs[par][e] = jnp.broadcast_to(src[:, 0:1], (8, 128))
                continue
            if r not in kf:
                kf[r] = pltpu.roll(kf_buf[g, j, r * 8:(r + 1) * 8, :], shift, 1)
            kbs[par][e] = jnp.broadcast_to(kf[r][:, d:d + 1], (8, 128))

    def attn_heads(it, carry):
        bad, carried = carry
        zero = it // H
        keep = lax.broadcasted_iota(jnp.int32, (8, 128), 0) >= zero
        ns = nc * nq
        o_init = jnp.full((dh, bq), zero, jnp.int32).astype(f32)
        l = {}
        o = {}
        pend, hist, marks = {}, [], []
        h0 = it * heads
        h_prev = jnp.maximum(h0 - 1, 0)
        for a in range(carry_over):
            n = a - carry_over
            pend[n] = carried[a][0].astype(bf16)
            l[-1, n % nq] = carried[a][1]
            o[-1, n % nq] = carried[a][2]
        carried = []
        for n in range(heads * ns + lag):
            z = zero * (n + 1)
            if n < heads * ns:
                u, (j, qb) = n // ns, divmod(n % ns, nq)
                h = h0 + u
                order = order_of(j)
                q = jnp.concatenate([qt_buf[h, qb * tq + t + z] for t in range(tq)], axis=1)
                kk = [kls[j % 2][a + z] for a in range(len(order))]
                if qtie and n >= qtie:
                    kk[0] = jnp.where(keep, kk[0], pltpu.bitcast(marks[n - qtie], u32))
                kk = pltpu.bitcast(jnp.concatenate(kk, axis=0), bf16)[:, :dh]
                s = _dot(kk, pltpu.bitcast(q, bf16))
                hist.append(s)
            m = n - lag
            do_pv = -carry_over <= m < heads * ns - carry_over
            if do_pv:
                uo, (jo, qo) = m // ns, divmod(m % ns, nq)
                ho = h_prev if uo < 0 else h0 + uo
                v = pltpu.bitcast(vt_buf[ho, jo + z], bf16)
                oc = _dot(v, pend.pop(m))
                o[uo, qo] = (o_init if jo == 0 and oinit else None if jo == 0 else o[uo, qo])
                o[uo, qo] = oc if o[uo, qo] is None else o[uo, qo] + oc
            if n < heads * ns:
                lq = l.get((u, qb))
                ps = [None] * (kc // 8)
                for k in range(2 * len(order)):
                    p = jnp.exp2(s[k * 8:(k + 1) * 8])
                    lq = p if lq is None else lq + p
                    ps[2 * order[k // 2] + k % 2] = p
                if j + 1 < nc:
                    stage(h, j + 1, (j + 1) % 2, qb, nq)
                else:
                    stage(jnp.minimum(h + 1, H - 1), 0, 0, qb, nq)
                for r0 in range(0, rv_of[j] // 8, kgb):
                    acc = [[None] * tq for _ in range(kgb)]
                    for d in range(dh):
                        kv = [kbs[j % 2][(r0 + a) * dh + d + z] for a in range(kgb)]
                        if tie and n >= tie and d % tie_d == 0:
                            hs = hist[n - tie]
                            ng = hs.shape[0] // 8
                            k = min(((r0 * dh + d * kgb) * ng) // (rv_of[j] // 8 * dh) + tie_off, ng - 1)
                            kv = [jnp.where(keep, x, hs[k * 8:(k + 1) * 8, :128]) for x in kv]
                        for t in range(tq):
                            qv = qv_buf[qb * tq + t, h * dh + d + zero * (4 * n + r0 // kgb + 1)]
                            for a in range(kgb):
                                pr = kv[a] * qv
                                acc[a][t] = pr if d == 0 else acc[a][t] + pr
                    for a in range(kgb):
                        p = jnp.exp2(jnp.concatenate(acc[a], axis=1))
                        ps[r0 + a] = p
                        lq = lq + p
                l[u, qb] = lq
                marks.append(p[:, :128])
                pf = jnp.concatenate(ps, axis=0)
                if n >= heads * ns - carry_over:
                    carried.append([pf, lq, None])
                else:
                    pend[n] = pf if pf32 else pf.astype(bf16)
            if do_pv and jo == nc - 1:
                bad = store_o(qo, ho, l[uo, qo], o[uo, qo], bad)
        for a in range(carry_over):
            carried[a][2] = o[heads - 1, (a - carry_over) % nq]
        return bad, tuple(tuple(c) for c in carried)

    if 2 in phases:
        stage(0, 0, 0, 0, 1)
        init = tuple((jnp.zeros((kc, bq), f32), jnp.ones((8, bq), f32), jnp.zeros((dh, bq), f32))
                     for _ in range(carry_over))
        bad, carried = lax.fori_loop(0, H // heads, attn_heads, (jnp.zeros((8, bq), f32), init))
        for a, (pf, lq, oq) in enumerate(carried):
            oq = oq + _dot(pltpu.bitcast(vt_buf[H - 1, nc - 1], bf16), pf.astype(bf16))
            bad = store_o(nq - carry_over + a, H - 1, lq, oq, bad)

        @pl.when(jnp.max(bad) > 0.0)
        def _():
            def body(n, _):
                h, t = n // (S // 128), n % (S // 128)
                kk = pltpu.roll(k_buf[h // hpg], (128 - (h % hpg) * dh) % 128, 1)
                s = _dot(pltpu.bitcast(kk, bf16)[:, :dh], pltpu.bitcast(qt_buf[h, t], bf16))
                p = jnp.exp2(s - jnp.max(s, axis=0, keepdims=True))
                v = jnp.concatenate([vt_buf[h, j] for j in range(S // 128)], axis=1)
                o = _dot(pltpu.bitcast(v, bf16), p.astype(bf16))
                ot_buf[t, pl.ds(pl.multiple_of(h * dh, dh), dh), :] = o * (1.0 / jnp.sum(p, axis=0, keepdims=True))
                return None

            lax.fori_loop(0, H * (S // 128), body, None)

    if 8 in phases:
        def dummy(n, acc):
            return (acc + qv_buf[n, n] + kf_buf[0, n, :8] + pltpu.bitcast(qt_buf[n, n] ^ vt_buf[n, n] ^ k_buf[n, :8], f32)
                    + t1[0, pl.ds(n * 16, 16), :128].astype(f32)[:8] + t2[0, pl.ds(n * 16, 16), :128].astype(f32)[:8])
        ot_buf[0, :8, :] = lax.fori_loop(0, 4, dummy, jnp.zeros((8, 128), f32))
        out_buf[:16, :128] = ot_buf[0, :16, :].astype(bf16)

    done = prep_in_b if (st_f and 1 in phases) else 0
    for c in (w1_copy, w2_copy)[done:] + (wo_copy, b1_copy, b2_copy):
        c.wait()

    def mlp_block(i, _):
        b1v = b1[pl.ds(0, F)].astype(f32).reshape(1, F)
        b2v = b2[pl.ds(0, D)].astype(f32).reshape(1, D)
        ns = bm3 // sub3
        hs, lns = [], []
        for s in range(ns):
            r0 = pl.multiple_of(i * bm3 + s * sub3, sub3)
            o = jnp.concatenate([ot_buf[r0 // 128 + t].T for t in range(sub3 // 128)], axis=0)
            h = x_buf[pl.ds(r0, sub3), :].astype(f32) + jnp.concatenate(_matmul(o, wo, to if st_o else None), axis=1)
            hs.append(h)
            lns.append(_layernorm(h))
        for s in range(ns):
            r0 = pl.multiple_of(i * bm3 + s * sub3, sub3)
            if not st_f:
                acc = hs[s] + b2v
                prev = None
                nfc = F // fc
                ln = lns[s].astype(bf16)
                for c in range(nfc + 1):
                    if c < nfc:
                        cols = slice(c * fc, (c + 1) * fc)
                        cur = _gelu(_dot(ln, w1[:, cols]) + b1v[:, cols]).astype(bf16)
                    if prev is not None:
                        acc = acc + _dot(prev, w2[(c - 1) * fc:c * fc, :])
                    prev = cur
            else:
                mh, dn, fh = sub3 // 2, D // 2, F // 2
                ln = lns[s]
                lhs1 = _strassen_lhs(ln[:mh, :dn], ln[:mh, dn:], ln[mh:, :dn], ln[mh:, dn:])
                accs = [None] * 7
                prev = None
                chunks = [slice(c, min(c + fc, fh)) for c in range(0, fh, fc)]
                for c in range(len(chunks) + 1):
                    cur = None
                    if c < len(chunks):
                        cols = chunks[c]
                        cols2 = slice(fh + cols.start, fh + cols.stop)
                        c11, c12, c21, c22 = _strassen_out(
                            [_dot(a, b) for a, b in zip(lhs1, _rhs_blocks(w1, t1, slice(0, dn), cols))])
                        cur = _strassen_lhs(_gelu(c11 + b1v[:, cols]), _gelu(c12 + b1v[:, cols2]),
                                            _gelu(c21 + b1v[:, cols]), _gelu(c22 + b1v[:, cols2]))
                    if prev is not None:
                        for n, (a, b) in enumerate(zip(prev, _rhs_blocks(w2, t2, chunks[c - 1], slice(0, dn)))):
                            accs[n] = _dot(a, b) if accs[n] is None else accs[n] + _dot(a, b)
                    prev = cur
                c11, c12, c21, c22 = _strassen_out(accs)
                y = jnp.concatenate([jnp.concatenate([c11, c12], axis=1), jnp.concatenate([c21, c22], axis=1)], axis=0)
                acc = hs[s] + b2v + y
            out_buf[pl.ds(r0, sub3), :] = acc.astype(bf16)
            out_copy(i * ns + s).start()
        return None

    def prep(w_ref, t_ref):
        def body(i, _):
            _strassen_rhs(w_ref, t_ref, pl.multiple_of(i * 32, 32), 32)
            return None
        lax.fori_loop(0, w_ref.shape[0] // 64, body, None)

    if 3 in phases:
        if st_o:
            prep(wo, to)
        if st_f and done < 1:
            prep(w1, t1)
        if st_f and done < 2:
            prep(w2, t2)
        lax.fori_loop(0, S // bm3, mlp_block, None)
    else:
        if 8 not in phases:
            out_buf[...] = jnp.zeros(out_buf.shape, bf16)
        for i in range(S // sub3):
            out_copy(i).start()
    for i in range(S // sub3):
        out_copy(i).wait()


DEFAULTS = dict(bq=512, kc=128, bma=2048, suba=128, bmb=512, subb=128, bm3=512, sub3=256, fc=256, lag=2,
                phases=(1, 2, 3), rv=16, kgb=1, heads=4, tie=2, tie_d=4, qtie=0, tie_off=0, carry_over=0,
                st_q=False, st_kv=False, st_o=False, st_f=True, xparts=(640, 2048), prep_in_b=1,
                rvs=None, ncb=128, fill_lead=0, atie=0, after_mode=1, late_w=1, oinit=True, pf32=False, rollb=False)


def make(variant="", flags=None, **kw):
    cfg = dict(DEFAULTS)
    cfg.update(kw)
    cfg["phases"] = tuple(cfg["phases"])
    if cfg["bma"] < 2048:
        cfg["xparts"] = tuple(range(cfg["bma"], 2049, cfg["bma"]))
    if cfg["rvs"]:
        cfg["rv"] = max(cfg["rvs"])

    def f(A_x, A_wqkv, A_wo, B_x, B_w1, B_b1, B_w2, B_b2):
        del B_x
        _, S, D = A_x.shape
        F = B_w1.shape[1]
        rv, kc = cfg["rv"], cfg["kc"]
        any_spec = pl.BlockSpec(memory_space=pl.ANY)
        return pl.pallas_call(
            functools.partial(_kernel, S=S, D=D, F=F, **cfg),
            in_specs=[any_spec] * 7,
            out_specs=any_spec,
            out_shape=jax.ShapeDtypeStruct(A_x.shape, A_x.dtype),
            scratch_shapes=[
                pltpu.VMEM((S, D), bf16), pltpu.VMEM((D, D), bf16), pltpu.VMEM((D, 2 * D), bf16),
                pltpu.VMEM((D, D), bf16),
                pltpu.VMEM((D, F), bf16), pltpu.VMEM((8192,), bf16), pltpu.VMEM((F, D), bf16), pltpu.VMEM((8192,), bf16),
                pltpu.VMEM((S, D), bf16), pltpu.VMEM((S, D), f32 if cfg["st_kv"] else bf16),
                pltpu.VMEM((D // 128, S // 2, 128), u32), pltpu.VMEM((H, S // 128, 8, 128), u32),
                pltpu.VMEM((H, S // 128, 8, 128), u32), pltpu.VMEM((S // 128, D, 128), f32),
                pltpu.VMEM((D // 128, S // kc, max(rv, 8), 128), f32),
                pltpu.VMEM((S // 128, D, 8, 128), f32),
                *[pltpu.VMEM((max(rv // 8, 1) * 16, 8, 128), f32)] * 2,
                *[pltpu.VMEM((kc // 16, 8, 128), u32)] * 2,
                pltpu.VMEM((5, D // 2, D // 2), bf16), pltpu.VMEM((5, D // 2, D), bf16),
                pltpu.VMEM((5, D // 2, D // 2), bf16),
                pltpu.VMEM((5, D // 2, F // 2), bf16), pltpu.VMEM((5, F // 2, D // 2), bf16),
                pltpu.SemaphoreType.DMA((len(cfg["xparts"]),)), pltpu.SemaphoreType.DMA((7,)),
                pltpu.SemaphoreType.DMA((S // cfg["sub3"],)),
            ],
            compiler_params=pltpu.CompilerParams(vmem_limit_bytes=100 * 2**20, flags=flags),
            name=KNAME,
        )(A_x, A_wqkv, A_wo, B_w1, B_b1, B_w2, B_b2)
    return f


@jax.jit
def pallas_sequential_preLN__softmax_full_mha__dense_activation_gelu__prompt_kernel(
    A_x, A_wqkv, A_wo, B_x, B_w1, B_b1, B_w2, B_b2,
):
    return make()(A_x, A_wqkv, A_wo, B_x, B_w1, B_b1, B_w2, B_b2)
```

```python
import functools
import math

import jax
import jax.numpy as jnp
from jax import lax
from jax.experimental import pallas as pl
from jax.experimental.pallas import tpu as pltpu

f32, bf16, u32 = jnp.float32, jnp.bfloat16, jnp.uint32

HEADS = 32
EPS = 1e-5
SUM_MIN, SUM_MAX = 2.0 ** -40, 2.0 ** 60
FINITE_MAX = 3.0e38

BQ = 512
TQ = BQ // 128
KC = 128
KC_VPU = 16
PV_LAG = 2
HEADS_PER_ITER = 4
D_GROUP = 4
X_FIRST = 768
MLP_ROWS = 256
MLP_COLS = 384


def _layernorm(x):
    mu = jnp.mean(x, axis=-1, keepdims=True)
    xc = x - mu
    var = jnp.mean(xc * xc, axis=-1, keepdims=True)
    return xc * lax.rsqrt(var + EPS)


def _gelu(x):
    c = math.sqrt(2.0 / math.pi)
    u = x * (c + (c * 0.044715) * (x * x))
    hx = 0.5 * x
    return hx + hx * jnp.tanh(u)


def _dot(a, b):
    return jnp.dot(a, b, preferred_element_type=f32)


def _all_true(zero):
    return lax.broadcasted_iota(jnp.int32, (8, 128), 0) >= zero


def _strassen_weight_sums(w_ref, t_ref, row, n, keep=None, after=None):
    kh, nh = w_ref.shape[0] // 2, w_ref.shape[1] // 2
    top = w_ref[pl.ds(row, n), :].astype(f32)
    bot = w_ref[pl.ds(kh + row, n), :].astype(f32)
    b11, b12, b21, b22 = top[:, :nh], top[:, nh:], bot[:, :nh], bot[:, nh:]
    if after is not None:
        reps = (n // 8, nh // 128)
        b11 = jnp.where(jnp.tile(keep, reps), b11, jnp.tile(after, reps))
        b22 = jnp.where(jnp.tile(keep, reps), b22, jnp.tile(after, reps))
    for i, t in enumerate((b11 + b22, b12 - b22, b21 - b11, b11 + b12, b21 + b22)):
        t_ref[i, pl.ds(row, n), :] = t.astype(bf16)


def _strassen_rhs(w_ref, t_ref, rows, cols):
    kh, nh = w_ref.shape[0] // 2, w_ref.shape[1] // 2
    rows2 = slice(kh + rows.start, kh + rows.stop)
    cols2 = slice(nh + cols.start, nh + cols.stop)
    return [t_ref[0, rows, cols], w_ref[rows, cols], t_ref[1, rows, cols], t_ref[2, rows, cols],
            w_ref[rows2, cols2], t_ref[3, rows, cols], t_ref[4, rows, cols]]


def _strassen_lhs(a11, a12, a21, a22):
    return [t.astype(bf16) for t in (a11 + a22, a21 + a22, a11, a22, a11 + a12, a21 - a11, a12 - a22)]


def _strassen_result(m):
    return m[0] + m[3] - m[4] + m[6], m[2] + m[4], m[1] + m[3], m[0] - m[1] + m[2] + m[5]


def _kernel(x_hbm, wqkv_hbm, wo_hbm, w1_hbm, b1_hbm, w2_hbm, b2_hbm, out_hbm,
            x_buf, wq, wkv, wo, w1, b1, w2, b2, out_buf, ln_buf,
            k_buf, qt_buf, vt_buf, ot_buf, kf_buf, qv_buf, kb0, kb1, kh0, kh1, t1, t2, sems):
    S, D = x_buf.shape
    F = w1.shape[1]
    dh = D // HEADS
    heads_per_group = 128 // dh
    nq, nc = S // BQ, S // KC
    q_scale = dh ** -0.5 * math.log2(math.e)

    def copy(src, dst, sem):
        return pltpu.make_async_copy(src, dst, sems.at[sem])

    def out_copy(i):
        rows = pl.ds(pl.multiple_of(i * MLP_ROWS, MLP_ROWS), MLP_ROWS)
        return copy(out_buf.at[rows], out_hbm.at[0, rows], 6)

    x_head = copy(x_hbm.at[0, pl.ds(0, X_FIRST)], x_buf.at[pl.ds(0, X_FIRST)], 0)
    x_tail = copy(x_hbm.at[0, pl.ds(X_FIRST, S - X_FIRST)], x_buf.at[pl.ds(X_FIRST, S - X_FIRST)], 1)
    wq_copy = copy(wqkv_hbm.at[:, pl.ds(0, D)], wq, 2)
    wkv_copy = copy(wqkv_hbm.at[:, pl.ds(D, 2 * D)], wkv, 3)
    w1_copy = copy(w1_hbm, w1, 4)
    mlp_copies = [copy(w2_hbm, w2, 5), copy(wo_hbm, wo, 5),
                  copy(b1_hbm, b1.at[pl.ds(0, F)], 5), copy(b2_hbm, b2.at[pl.ds(0, D)], 5)]
    for c in (x_head, wq_copy, x_tail, wkv_copy):
        c.start()

    def norm_rows(r):
        ln = _layernorm(x_buf[pl.ds(r, 128), :].astype(f32)).astype(bf16)
        ln_buf[pl.ds(r, 128), :] = ln
        return ln

    def project_q(r, ln):
        qt = pltpu.bitcast((_dot(ln, wq[...]) * q_scale).T.astype(bf16), u32)
        qt_buf[:, r // BQ, r % BQ // 128] = qt.reshape(HEADS, 8, 128)

    ln = {}
    x_head.wait()
    for r in range(0, 256, 128):
        ln[r] = norm_rows(r)
    wq_copy.wait()
    for r in range(256, X_FIRST, 128):
        ln[r] = norm_rows(r)
    for r in range(0, X_FIRST - 128, 128):
        project_q(r, ln[r])
    x_tail.wait()
    for r in range(X_FIRST, S, 128):
        ln[r] = norm_rows(r)
    for r in range(X_FIRST - 128, S, 128):
        project_q(r, ln[r])
    for c in (w1_copy, *mlp_copies):
        c.start()
    wkv_copy.wait()
    w1_copy.wait()

    def project_kv(i, _):
        keep = _all_true(i // S)

        def replicate_q(t, h, after):
            q = jnp.where(keep, qt_buf[h, i, t], pltpu.bitcast(after, u32))
            q = pltpu.bitcast(q, bf16).astype(f32)
            rows = [jnp.broadcast_to(q[d:d + 1], (8, 128)) for d in range(dh)]
            qv_buf[i, pl.ds(h * dh, dh), :, t * 128:(t + 1) * 128] = jnp.stack(rows)

        fill = [functools.partial(replicate_q, t, h) for t in range(TQ) for h in range(HEADS)]
        w1_rows = D // 2 // nq
        for n, r in enumerate(range(0, w1_rows, 16)):
            fill.insert(n * (len(fill) * 16 // w1_rows), functools.partial(
                _strassen_weight_sums, w1, t1, pl.multiple_of(i * w1_rows + r, 16), 16, keep))
        n_dots = TQ * (2 * D // 128)
        dots_done, fill_done = 0, 0

        def dot_and_fill(a, b):
            nonlocal dots_done, fill_done
            y = _dot(a, b)
            dots_done += 1
            last = min((dots_done + 1) * len(fill) // n_dots, len(fill))
            for n in range(fill_done, last):
                r = (n - fill_done) * (y.shape[0] // 8) // (last - fill_done) * 8
                fill[n](y[r:r + 8, :128])
            fill_done = last
            return y

        for t in range(TQ):
            blk = i * TQ + t
            a = ln_buf[pl.ds(pl.multiple_of(blk * 128, 128), 128), :]
            v = jnp.concatenate([dot_and_fill(a, wkv[:, D + c:D + c + 128]) for c in range(0, D, 128)], axis=1)
            k = jnp.concatenate([dot_and_fill(a, wkv[:, c:c + 128]) for c in range(0, D, 128)], axis=1)
            k = k.astype(bf16)
            vt_buf[:, i, t] = pltpu.bitcast(v.T.astype(bf16), u32).reshape(HEADS, 8, 128)
            k_packed = pltpu.bitcast(k, u32)
            for g in range(D // 128):
                k_buf[g, blk] = k_packed[:, g * 128:(g + 1) * 128]
                kf_buf[g, i, t] = k[:KC_VPU, g * 128:(g + 1) * 128].astype(f32)
        return None

    lax.fori_loop(0, nq, project_kv, None)

    k_heads, k_bcast = (kh0, kh1), (kb0, kb1)
    n_kh = (KC - KC_VPU) // 16
    n_kb = KC_VPU // 8 * dh

    def head_shift(h):
        return (128 - (h % heads_per_group) * dh) % 128

    def stage_keys(h, j, part, parts):
        g, shift = h // heads_per_group, head_shift(h)
        for a in range(part * n_kh // parts, (part + 1) * n_kh // parts):
            r = (KC_VPU + a * 16) // 2
            k_heads[j % 2][a] = pltpu.roll(k_buf[g, j, r:r + 8], shift, 1)
        kf = {}
        for e in range(part * n_kb // parts, (part + 1) * n_kb // parts):
            r, d = divmod(e, dh)
            if r not in kf:
                kf[r] = pltpu.roll(kf_buf[g, j // TQ, j % TQ, r * 8:(r + 1) * 8, :], shift, 1)
            k_bcast[j % 2][e] = jnp.broadcast_to(kf[r][:, d:d + 1], (8, 128))

    def attend_unshifted(it, unsafe):
        zero = it // HEADS
        keep = _all_true(zero)
        o_zero = jnp.full((dh, BQ), zero, jnp.int32).astype(f32)
        per_head = nc * nq
        steps = HEADS_PER_ITER * per_head
        rows_mxu = 2 * n_kh
        groups = n_kb // D_GROUP
        sums, outs, probs, scores = {}, {}, {}, []
        for n in range(steps + PV_LAG):
            z = zero * (n + 1)
            if n < steps:
                u, (j, qb) = n // per_head, divmod(n % per_head, nq)
                h = it * HEADS_PER_ITER + u
                q = jnp.concatenate([qt_buf[h, qb + z, t] for t in range(TQ)], axis=1)
                k = k_heads[j % 2][pl.ds(z, n_kh)].reshape(n_kh * 8, 128)
                scores.append(_dot(pltpu.bitcast(k, bf16)[:, :dh], pltpu.bitcast(q, bf16)))
            if n >= PV_LAG:
                uo, (jo, qo) = (n - PV_LAG) // per_head, divmod((n - PV_LAG) % per_head, nq)
                v = vt_buf[it * HEADS_PER_ITER + uo, jo // TQ + z, jo % TQ]
                pv = _dot(pltpu.bitcast(v, bf16), probs.pop(n - PV_LAG))
                outs[qo] = (o_zero if jo == 0 else outs[qo]) + pv
            if n < steps:
                p_mxu = jnp.exp2(scores[n])
                if j + 1 < nc:
                    stage_keys(h, j + 1, qb, nq)
                else:
                    stage_keys(jnp.minimum(h + 1, HEADS - 1), 0, qb, nq)
                p_vpu = []
                for r in range(KC_VPU // 8):
                    s = None
                    for d in range(0, dh, D_GROUP):
                        qv = qv_buf[qb, pl.ds(h * dh + d + zero * (4 * n + r + 1), D_GROUP)]
                        kv = k_bcast[j % 2][pl.ds(r * dh + d + z, D_GROUP)]
                        pos = (n - 1) * rows_mxu + (r * dh + d) // D_GROUP * rows_mxu // groups + 3
                        if pos >= 0:
                            step, row = divmod(pos, rows_mxu)
                            first = jnp.where(keep, kv[0], scores[step][row * 8:(row + 1) * 8, :128])
                            kv = jnp.concatenate([first[None], kv[1:]], axis=0)
                        prod = jnp.concatenate([kv] * TQ, axis=2) * qv
                        for c in range(D_GROUP):
                            s = prod[c] if s is None else s + prod[c]
                    p_vpu.append(jnp.exp2(s))
                total = sums[u, qb] if j else None
                rows = [p_mxu[r * 8:(r + 1) * 8] for r in range(rows_mxu)]
                for p in rows[:10] + p_vpu + rows[10:]:
                    total = p if total is None else total + p
                sums[u, qb] = total
                probs[n] = jnp.concatenate(p_vpu + [p_mxu], axis=0).astype(bf16)
            if n >= PV_LAG and jo == nc - 1:
                total = jnp.sum(sums[uo, qo], axis=0, keepdims=True)
                o = outs[qo] * (1.0 / total)
                pair, odd = it * (HEADS_PER_ITER // 2) + uo // 2, uo % 2
                for t in range(TQ):
                    ot_buf[qo * TQ + t, pair, odd * dh:(odd + 1) * dh, :] = o[:, t * 128:(t + 1) * 128]
                safe = ((total >= SUM_MIN) & (total <= SUM_MAX)
                        & (jnp.abs(o[:8]) + jnp.abs(o[8:]) <= FINITE_MAX))
                unsafe = jnp.where(safe, unsafe, 1.0)
        return unsafe

    def attend_with_max(n, _):
        h, qb = n // nq, n % nq
        q = pltpu.bitcast(jnp.concatenate([qt_buf[h, qb, t] for t in range(TQ)], axis=1), bf16)
        rows = BQ // 8

        def row_max(c, m):
            k = k_buf[h // heads_per_group, pl.ds(c * TQ, TQ)].reshape(BQ // 2, 128)
            k = pltpu.bitcast(pltpu.roll(k, head_shift(h), 1), bf16)
            s = _dot(k[:, :dh], q).reshape(rows, 8, BQ)
            qv_buf[0, pl.ds(c * rows, rows)] = s
            return jnp.maximum(m, jnp.max(s, axis=0))

        m = lax.fori_loop(0, S // BQ, row_max, jnp.full((8, BQ), -jnp.inf, f32))
        m = jnp.max(m, axis=0, keepdims=True)

        def accumulate(c, acc):
            p = jnp.exp2(qv_buf[0, pl.ds(c * rows, rows)] - m)
            v = jnp.concatenate([vt_buf[h, c, t] for t in range(TQ)], axis=1)
            return (acc[0] + jnp.sum(p, axis=0),
                    acc[1] + _dot(pltpu.bitcast(v, bf16), p.reshape(BQ, BQ).astype(bf16)))

        total, o = lax.fori_loop(0, S // BQ, accumulate, (jnp.zeros((8, BQ), f32), jnp.zeros((dh, BQ), f32)))
        o = o * (1.0 / jnp.sum(total, axis=0, keepdims=True))
        for t in range(TQ):
            ot_buf[qb * TQ + t, h // 2, pl.ds(pl.multiple_of(h % 2 * dh, dh), dh), :] = o[:, t * 128:(t + 1) * 128]
        return None

    stage_keys(0, 0, 0, 1)
    unsafe = lax.fori_loop(0, HEADS // HEADS_PER_ITER, attend_unshifted, jnp.zeros((8, BQ), f32))

    @pl.when(jnp.max(unsafe) > 0.0)
    def _():
        lax.fori_loop(0, HEADS * nq, attend_with_max, None)

    for c in mlp_copies:
        c.wait()

    def w2_sums(i, _):
        _strassen_weight_sums(w2, t2, pl.multiple_of(i * 64, 64), 64)
        return None

    lax.fori_loop(0, F // 2 // 64, w2_sums, None)

    def mlp(i, _):
        bias1 = b1[pl.ds(0, F)].astype(f32).reshape(1, F)
        bias2 = b2[pl.ds(0, D)].astype(f32).reshape(1, D)
        starts = [pl.multiple_of(i * BQ + r, MLP_ROWS) for r in range(0, BQ, MLP_ROWS)]
        hs, lns = [], []
        for r in starts:
            o = [ot_buf[r // 128 + t].reshape(D, 128).T for t in range(MLP_ROWS // 128)]
            o = jnp.concatenate(o, axis=0)
            h = x_buf[pl.ds(r, MLP_ROWS), :].astype(f32) + _dot(o.astype(bf16), wo[...])
            hs.append(h)
            lns.append(_layernorm(h))
        mh, kh, fh = MLP_ROWS // 2, D // 2, F // 2
        chunks = [slice(c, min(c + MLP_COLS, fh)) for c in range(0, fh, MLP_COLS)]
        for n, (r, h, a) in enumerate(zip(starts, hs, lns)):
            lhs = _strassen_lhs(a[:mh, :kh], a[:mh, kh:], a[mh:, :kh], a[mh:, kh:])
            acc = [None] * 7
            prev = None
            for c in range(len(chunks) + 1):
                cur = None
                if c < len(chunks):
                    left = chunks[c]
                    right = slice(fh + left.start, fh + left.stop)
                    c11, c12, c21, c22 = _strassen_result(
                        [_dot(y, w) for y, w in zip(lhs, _strassen_rhs(w1, t1, slice(0, kh), left))])
                    cur = _strassen_lhs(_gelu(c11 + bias1[:, left]), _gelu(c12 + bias1[:, right]),
                                        _gelu(c21 + bias1[:, left]), _gelu(c22 + bias1[:, right]))
                if prev is not None:
                    for b, (y, w) in enumerate(zip(prev, _strassen_rhs(w2, t2, chunks[c - 1], slice(0, kh)))):
                        acc[b] = _dot(y, w) if acc[b] is None else acc[b] + _dot(y, w)
                prev = cur
            c11, c12, c21, c22 = _strassen_result(acc)
            y = jnp.concatenate([jnp.concatenate([c11, c12], axis=1), jnp.concatenate([c21, c22], axis=1)], axis=0)
            out_buf[pl.ds(r, MLP_ROWS), :] = (h + bias2 + y).astype(bf16)
            out_copy(i * len(starts) + n).start()
        return None

    lax.fori_loop(0, nq, mlp, None)
    for i in range(S // MLP_ROWS):
        out_copy(i).wait()


@jax.jit
def pallas_sequential_preLN__softmax_full_mha__dense_activation_gelu__prompt_kernel(
    A_x: jax.Array,
    A_wqkv: jax.Array,
    A_wo: jax.Array,
    B_x: jax.Array,
    B_w1: jax.Array,
    B_b1: jax.Array,
    B_w2: jax.Array,
    B_b2: jax.Array,
):
    del B_x
    batch, S, D = A_x.shape
    F = B_w1.shape[1]
    assert (batch, S, D, F) == (1, 2048, 512, 1792)
    dh = D // HEADS
    vmem = pltpu.VMEM
    in_hbm = pl.BlockSpec(memory_space=pl.ANY)
    return pl.pallas_call(
        _kernel,
        in_specs=[in_hbm] * 7,
        out_specs=in_hbm,
        out_shape=jax.ShapeDtypeStruct(A_x.shape, A_x.dtype),
        scratch_shapes=[
            vmem((S, D), bf16),
            vmem((D, D), bf16),
            vmem((D, 2 * D), bf16),
            vmem((D, D), bf16),
            vmem((D, F), bf16),
            vmem((8192,), bf16),
            vmem((F, D), bf16),
            vmem((8192,), bf16),
            vmem((S, D), bf16),
            vmem((S, D), bf16),
            vmem((D // 128, S // KC, KC // 2, 128), u32),
            vmem((HEADS, S // BQ, TQ, dh // 2, 128), u32),
            vmem((HEADS, S // BQ, TQ, dh // 2, 128), u32),
            vmem((S // 128, HEADS // 2, 2 * dh, 128), f32),
            vmem((D // 128, S // BQ, TQ, KC_VPU, 128), f32),
            vmem((S // BQ, D, 8, BQ), f32),
            vmem((KC_VPU // 8 * dh, 8, 128), f32),
            vmem((KC_VPU // 8 * dh, 8, 128), f32),
            vmem((KC // 16, 8, 128), u32),
            vmem((KC // 16, 8, 128), u32),
            vmem((5, D // 2, F // 2), bf16),
            vmem((5, F // 2, D // 2), bf16),
            pltpu.SemaphoreType.DMA((7,)),
        ],
        compiler_params=pltpu.CompilerParams(vmem_limit_bytes=96 * 2**20),
        name="fused_block",
    )(A_x, A_wqkv, A_wo, B_w1, B_b1, B_w2, B_b2)
```

```python
import functools
import math

import jax
import jax.numpy as jnp
from jax import lax
from jax.experimental import pallas as pl
from jax.experimental.pallas import tpu as pltpu

f32, bf16, u32 = jnp.float32, jnp.bfloat16, jnp.uint32

HEADS = 32
EPS = 1e-5
SUM_MIN, SUM_MAX = 2.0 ** -40, 2.0 ** 60
FINITE_MAX = 3.0e38

BQ = 512
TQ = BQ // 128
KC = 128
KC_VPU = 16
PV_LAG = 2
HEADS_PER_ITER = 4
D_GROUP = 4
X_FIRST = 768
MLP_ROWS = 256
MLP_COLS = 384


def _layernorm(x):
    mu = jnp.mean(x, axis=-1, keepdims=True)
    xc = x - mu
    var = jnp.mean(xc * xc, axis=-1, keepdims=True)
    return xc * lax.rsqrt(var + EPS)


def _gelu(x):
    c = math.sqrt(2.0 / math.pi)
    u = x * (c + (c * 0.044715) * (x * x))
    hx = 0.5 * x
    return hx + hx * jnp.tanh(u)


def _dot(a, b):
    return jnp.dot(a, b, preferred_element_type=f32)


def _all_true(zero):
    return lax.broadcasted_iota(jnp.int32, (8, 128), 0) >= zero


def _strassen_weight_sums(w_ref, t_ref, row, n, keep=None, after=None):
    kh, nh = w_ref.shape[0] // 2, w_ref.shape[1] // 2
    top = w_ref[pl.ds(row, n), :].astype(f32)
    bot = w_ref[pl.ds(kh + row, n), :].astype(f32)
    b11, b12, b21, b22 = top[:, :nh], top[:, nh:], bot[:, :nh], bot[:, nh:]
    if after is not None:
        reps = (n // 8, nh // 128)
        b11 = jnp.where(jnp.tile(keep, reps), b11, jnp.tile(after, reps))
        b22 = jnp.where(jnp.tile(keep, reps), b22, jnp.tile(after, reps))
    for i, t in enumerate((b11 + b22, b12 - b22, b21 - b11, b11 + b12, b21 + b22)):
        t_ref[i, pl.ds(row, n), :] = t.astype(bf16)


def _strassen_rhs(w_ref, t_ref, rows, cols):
    kh, nh = w_ref.shape[0] // 2, w_ref.shape[1] // 2
    rows2 = slice(kh + rows.start, kh + rows.stop)
    cols2 = slice(nh + cols.start, nh + cols.stop)
    return [t_ref[0, rows, cols], w_ref[rows, cols], t_ref[1, rows, cols], t_ref[2, rows, cols],
            w_ref[rows2, cols2], t_ref[3, rows, cols], t_ref[4, rows, cols]]


def _strassen_lhs(a11, a12, a21, a22):
    return [t.astype(bf16) for t in (a11 + a22, a21 + a22, a11, a22, a11 + a12, a21 - a11, a12 - a22)]


def _strassen_result(m):
    return m[0] + m[3] - m[4] + m[6], m[2] + m[4], m[1] + m[3], m[0] - m[1] + m[2] + m[5]


def _kernel(x_hbm, wqkv_hbm, wo_hbm, w1_hbm, b1_hbm, w2_hbm, b2_hbm, out_hbm,
            x_buf, wq, wkv, wo, w1, b1, w2, b2, out_buf, ln_buf,
            k_buf, qt_buf, vt_buf, ot_buf, kf_buf, qv_buf, kb0, kb1, kh0, kh1, t1, t2, sems):
    S, D = x_buf.shape
    F = w1.shape[1]
    dh = D // HEADS
    heads_per_group = 128 // dh
    nq, nc = S // BQ, S // KC
    q_scale = dh ** -0.5 * math.log2(math.e)

    def copy(src, dst, sem):
        return pltpu.make_async_copy(src, dst, sems.at[sem])

    def out_copy(i):
        rows = pl.ds(pl.multiple_of(i * MLP_ROWS, MLP_ROWS), MLP_ROWS)
        return copy(out_buf.at[rows], out_hbm.at[0, rows], 6)

    x_head = copy(x_hbm.at[0, pl.ds(0, X_FIRST)], x_buf.at[pl.ds(0, X_FIRST)], 0)
    x_tail = copy(x_hbm.at[0, pl.ds(X_FIRST, S - X_FIRST)], x_buf.at[pl.ds(X_FIRST, S - X_FIRST)], 1)
    wq_copy = copy(wqkv_hbm.at[:, pl.ds(0, D)], wq, 2)
    wkv_copy = copy(wqkv_hbm.at[:, pl.ds(D, 2 * D)], wkv, 3)
    w1_copy = copy(w1_hbm, w1, 4)
    mlp_copies = [copy(w2_hbm, w2, 5), copy(wo_hbm, wo, 5),
                  copy(b1_hbm, b1.at[pl.ds(0, F)], 5), copy(b2_hbm, b2.at[pl.ds(0, D)], 5)]
    for c in (x_head, wq_copy, x_tail, wkv_copy):
        c.start()

    def norm_rows(r):
        ln = _layernorm(x_buf[pl.ds(r, 128), :].astype(f32)).astype(bf16)
        ln_buf[pl.ds(r, 128), :] = ln
        return ln

    def project_q(r, ln):
        qt = pltpu.bitcast((_dot(ln, wq[...]) * q_scale).T.astype(bf16), u32)
        qt_buf[:, r // BQ, r % BQ // 128] = qt.reshape(HEADS, 8, 128)

    ln = {}
    x_head.wait()
    for r in range(0, 256, 128):
        ln[r] = norm_rows(r)
    wq_copy.wait()
    for r in range(256, X_FIRST, 128):
        ln[r] = norm_rows(r)
    for r in range(0, X_FIRST - 128, 128):
        project_q(r, ln[r])
    x_tail.wait()
    for r in range(X_FIRST, S, 128):
        ln[r] = norm_rows(r)
    for r in range(X_FIRST - 128, S, 128):
        project_q(r, ln[r])
    for c in (w1_copy, *mlp_copies):
        c.start()
    wkv_copy.wait()
    w1_copy.wait()

    def project_kv(i, _):
        keep = _all_true(i // S)

        def replicate_q(t, h, after):
            q = jnp.where(keep, qt_buf[h, i, t], pltpu.bitcast(after, u32))
            q = pltpu.bitcast(q, bf16).astype(f32)
            rows = [jnp.broadcast_to(q[d:d + 1], (8, 128)) for d in range(dh)]
            qv_buf[i, pl.ds(h * dh, dh), :, t * 128:(t + 1) * 128] = jnp.stack(rows)

        fill = [functools.partial(replicate_q, t, h) for t in range(TQ) for h in range(HEADS)]
        w1_rows = D // 2 // nq
        for n, r in enumerate(range(0, w1_rows, 16)):
            fill.insert(n * (len(fill) * 16 // w1_rows), functools.partial(
                _strassen_weight_sums, w1, t1, pl.multiple_of(i * w1_rows + r, 16), 16, keep))
        n_dots = TQ * (2 * D // 128)
        dots_done, fill_done = 0, 0

        def dot_and_fill(a, b):
            nonlocal dots_done, fill_done
            y = _dot(a, b)
            dots_done += 1
            last = min((dots_done + 1) * len(fill) // n_dots, len(fill))
            for n in range(fill_done, last):
                r = (n - fill_done) * (y.shape[0] // 8) // (last - fill_done) * 8
                fill[n](y[r:r + 8, :128])
            fill_done = last
            return y

        for t in range(TQ):
            blk = i * TQ + t
            a = ln_buf[pl.ds(pl.multiple_of(blk * 128, 128), 128), :]
            v = jnp.concatenate([dot_and_fill(a, wkv[:, D + c:D + c + 128]) for c in range(0, D, 128)], axis=1)
            k = jnp.concatenate([dot_and_fill(a, wkv[:, c:c + 128]) for c in range(0, D, 128)], axis=1)
            k = k.astype(bf16)
            vt_buf[:, i, t] = pltpu.bitcast(v.T.astype(bf16), u32).reshape(HEADS, 8, 128)
            k_packed = pltpu.bitcast(k, u32)
            for g in range(D // 128):
                k_buf[g, blk] = k_packed[:, g * 128:(g + 1) * 128]
                kf_buf[g, i, t] = k[:KC_VPU, g * 128:(g + 1) * 128].astype(f32)
        return None

    lax.fori_loop(0, nq, project_kv, None)

    k_heads, k_bcast = (kh0, kh1), (kb0, kb1)
    n_kh = (KC - KC_VPU) // 16
    n_kb = KC_VPU // 8 * dh

    def head_shift(h):
        return (128 - (h % heads_per_group) * dh) % 128

    def stage_keys(h, j, part, parts):
        g, shift = h // heads_per_group, head_shift(h)
        lo, hi = part * n_kh // parts, (part + 1) * n_kh // parts
        k = pltpu.roll(k_buf[g, j, KC_VPU // 2 + lo * 8:KC_VPU // 2 + hi * 8], shift, 1)
        k_heads[j % 2][lo:hi] = k.reshape(hi - lo, 8, 128)
        lo, hi = part * n_kb // parts, (part + 1) * n_kb // parts
        r0, r1 = lo // dh, (hi - 1) // dh + 1
        k = pltpu.roll(kf_buf[g, j // TQ, j % TQ, r0 * 8:r1 * 8, :], shift, 1)
        cols = [k[(e // dh - r0) * 8:(e // dh - r0 + 1) * 8, e % dh:e % dh + 1] for e in range(lo, hi)]
        k_bcast[j % 2][lo:hi] = jnp.stack([jnp.broadcast_to(c, (8, 128)) for c in cols])

    def attend_unshifted(it, unsafe):
        zero = it // HEADS
        keep = _all_true(zero)
        o_zero = jnp.full((dh, BQ), zero, jnp.int32).astype(f32)
        per_head = nc * nq
        steps = HEADS_PER_ITER * per_head
        rows_mxu = 2 * n_kh
        groups = n_kb // D_GROUP
        sums, outs, probs, scores = {}, {}, {}, []
        for n in range(steps + PV_LAG):
            z = zero * (n + 1)
            if n < steps:
                u, (j, qb) = n // per_head, divmod(n % per_head, nq)
                h = it * HEADS_PER_ITER + u
                q = qt_buf[h, qb + z]
                q = jnp.concatenate([q[t] for t in range(TQ)], axis=1)
                k = k_heads[j % 2][pl.ds(z, n_kh)].reshape(n_kh * 8, 128)
                scores.append(_dot(pltpu.bitcast(k, bf16)[:, :dh], pltpu.bitcast(q, bf16)))
            if n >= PV_LAG:
                uo, (jo, qo) = (n - PV_LAG) // per_head, divmod((n - PV_LAG) % per_head, nq)
                v = vt_buf[it * HEADS_PER_ITER + uo, jo // TQ + z, jo % TQ]
                pv = _dot(pltpu.bitcast(v, bf16), probs.pop(n - PV_LAG))
                outs[qo] = (o_zero if jo == 0 else outs[qo]) + pv
            if n < steps:
                p_mxu = jnp.exp2(scores[n])
                if j + 1 < nc:
                    stage_keys(h, j + 1, qb, nq)
                else:
                    stage_keys(jnp.minimum(h + 1, HEADS - 1), 0, qb, nq)
                p_vpu = []
                k_cols = k_bcast[j % 2][pl.ds(z, n_kb)]
                for r in range(KC_VPU // 8):
                    s = None
                    q_rows = qv_buf[qb, pl.ds(h * dh + zero * (4 * n + r + 1), dh)]
                    for d in range(0, dh, D_GROUP):
                        qv = q_rows[d:d + D_GROUP]
                        kv = k_cols[r * dh + d:r * dh + d + D_GROUP]
                        pos = (n - 1) * rows_mxu + (r * dh + d) // D_GROUP * rows_mxu // groups + 3
                        if pos >= 0:
                            step, row = divmod(pos, rows_mxu)
                            first = jnp.where(keep, kv[0], scores[step][row * 8:(row + 1) * 8, :128])
                            kv = jnp.concatenate([first[None], kv[1:]], axis=0)
                        prod = jnp.concatenate([kv] * TQ, axis=2) * qv
                        for c in range(D_GROUP):
                            s = prod[c] if s is None else s + prod[c]
                    p_vpu.append(jnp.exp2(s))
                total = sums[u, qb] if j else None
                rows = [p_mxu[r * 8:(r + 1) * 8] for r in range(rows_mxu)]
                for p in rows[:10] + p_vpu + rows[10:]:
                    total = p if total is None else total + p
                sums[u, qb] = total
                probs[n] = jnp.concatenate(p_vpu + [p_mxu], axis=0).astype(bf16)
            if n >= PV_LAG and jo == nc - 1:
                total = jnp.sum(sums[uo, qo], axis=0, keepdims=True)
                o = outs[qo] * (1.0 / total)
                pair, odd = it * (HEADS_PER_ITER // 2) + uo // 2, uo % 2
                for t in range(TQ):
                    ot_buf[qo * TQ + t, pair, odd * dh:(odd + 1) * dh, :] = o[:, t * 128:(t + 1) * 128]
                safe = ((total >= SUM_MIN) & (total <= SUM_MAX)
                        & (jnp.abs(o[:8]) + jnp.abs(o[8:]) <= FINITE_MAX))
                unsafe = jnp.where(safe, unsafe, 1.0)
        return unsafe

    def attend_with_max(n, _):
        h, qb = n // nq, n % nq
        q = pltpu.bitcast(jnp.concatenate([qt_buf[h, qb, t] for t in range(TQ)], axis=1), bf16)
        rows = BQ // 8

        def row_max(c, m):
            k = k_buf[h // heads_per_group, pl.ds(c * TQ, TQ)].reshape(BQ // 2, 128)
            k = pltpu.bitcast(pltpu.roll(k, head_shift(h), 1), bf16)
            s = _dot(k[:, :dh], q).reshape(rows, 8, BQ)
            qv_buf[0, pl.ds(c * rows, rows)] = s
            return jnp.maximum(m, jnp.max(s, axis=0))

        m = lax.fori_loop(0, S // BQ, row_max, jnp.full((8, BQ), -jnp.inf, f32))
        m = jnp.max(m, axis=0, keepdims=True)

        def accumulate(c, acc):
            p = jnp.exp2(qv_buf[0, pl.ds(c * rows, rows)] - m)
            v = jnp.concatenate([vt_buf[h, c, t] for t in range(TQ)], axis=1)
            return (acc[0] + jnp.sum(p, axis=0),
                    acc[1] + _dot(pltpu.bitcast(v, bf16), p.reshape(BQ, BQ).astype(bf16)))

        total, o = lax.fori_loop(0, S // BQ, accumulate, (jnp.zeros((8, BQ), f32), jnp.zeros((dh, BQ), f32)))
        o = o * (1.0 / jnp.sum(total, axis=0, keepdims=True))
        for t in range(TQ):
            ot_buf[qb * TQ + t, h // 2, pl.ds(pl.multiple_of(h % 2 * dh, dh), dh), :] = o[:, t * 128:(t + 1) * 128]
        return None

    stage_keys(0, 0, 0, 1)
    unsafe = lax.fori_loop(0, HEADS // HEADS_PER_ITER, attend_unshifted, jnp.zeros((8, BQ), f32))

    @pl.when(jnp.max(unsafe) > 0.0)
    def _():
        lax.fori_loop(0, HEADS * nq, attend_with_max, None)

    for c in mlp_copies:
        c.wait()

    def w2_sums(i, _):
        _strassen_weight_sums(w2, t2, pl.multiple_of(i * 64, 64), 64)
        return None

    lax.fori_loop(0, F // 2 // 64, w2_sums, None)

    def mlp(i, _):
        bias1 = b1[pl.ds(0, F)].astype(f32).reshape(1, F)
        bias2 = b2[pl.ds(0, D)].astype(f32).reshape(1, D)
        starts = [pl.multiple_of(i * BQ + r, MLP_ROWS) for r in range(0, BQ, MLP_ROWS)]
        hs, lns = [], []
        for r in starts:
            o = [ot_buf[r // 128 + t].reshape(D, 128).T for t in range(MLP_ROWS // 128)]
            o = jnp.concatenate(o, axis=0)
            h = x_buf[pl.ds(r, MLP_ROWS), :].astype(f32) + _dot(o.astype(bf16), wo[...])
            hs.append(h)
            lns.append(_layernorm(h))
        mh, kh, fh = MLP_ROWS // 2, D // 2, F // 2
        chunks = [slice(c, min(c + MLP_COLS, fh)) for c in range(0, fh, MLP_COLS)]
        for n, (r, h, a) in enumerate(zip(starts, hs, lns)):
            lhs = _strassen_lhs(a[:mh, :kh], a[:mh, kh:], a[mh:, :kh], a[mh:, kh:])
            acc = [None] * 7
            prev = None
            for c in range(len(chunks) + 1):
                cur = None
                if c < len(chunks):
                    left = chunks[c]
                    right = slice(fh + left.start, fh + left.stop)
                    c11, c12, c21, c22 = _strassen_result(
                        [_dot(y, w) for y, w in zip(lhs, _strassen_rhs(w1, t1, slice(0, kh), left))])
                    cur = _strassen_lhs(_gelu(c11 + bias1[:, left]), _gelu(c12 + bias1[:, right]),
                                        _gelu(c21 + bias1[:, left]), _gelu(c22 + bias1[:, right]))
                if prev is not None:
                    for b, (y, w) in enumerate(zip(prev, _strassen_rhs(w2, t2, chunks[c - 1], slice(0, kh)))):
                        acc[b] = _dot(y, w) if acc[b] is None else acc[b] + _dot(y, w)
                prev = cur
            c11, c12, c21, c22 = _strassen_result(acc)
            y = jnp.concatenate([jnp.concatenate([c11, c12], axis=1), jnp.concatenate([c21, c22], axis=1)], axis=0)
            out_buf[pl.ds(r, MLP_ROWS), :] = (h + bias2 + y).astype(bf16)
            out_copy(i * len(starts) + n).start()
        return None

    lax.fori_loop(0, nq, mlp, None)
    for i in range(S // MLP_ROWS):
        out_copy(i).wait()


@jax.jit
def pallas_sequential_preLN__softmax_full_mha__dense_activation_gelu__prompt_kernel(
    A_x: jax.Array,
    A_wqkv: jax.Array,
    A_wo: jax.Array,
    B_x: jax.Array,
    B_w1: jax.Array,
    B_b1: jax.Array,
    B_w2: jax.Array,
    B_b2: jax.Array,
):
    del B_x
    batch, S, D = A_x.shape
    F = B_w1.shape[1]
    assert (batch, S, D, F) == (1, 2048, 512, 1792)
    dh = D // HEADS
    vmem = pltpu.VMEM
    in_hbm = pl.BlockSpec(memory_space=pl.ANY)
    return pl.pallas_call(
        _kernel,
        in_specs=[in_hbm] * 7,
        out_specs=in_hbm,
        out_shape=jax.ShapeDtypeStruct(A_x.shape, A_x.dtype),
        scratch_shapes=[
            vmem((S, D), bf16),
            vmem((D, D), bf16),
            vmem((D, 2 * D), bf16),
            vmem((D, D), bf16),
            vmem((D, F), bf16),
            vmem((8192,), bf16),
            vmem((F, D), bf16),
            vmem((8192,), bf16),
            vmem((S, D), bf16),
            vmem((S, D), bf16),
            vmem((D // 128, S // KC, KC // 2, 128), u32),
            vmem((HEADS, S // BQ, TQ, dh // 2, 128), u32),
            vmem((HEADS, S // BQ, TQ, dh // 2, 128), u32),
            vmem((S // 128, HEADS // 2, 2 * dh, 128), f32),
            vmem((D // 128, S // BQ, TQ, KC_VPU, 128), f32),
            vmem((S // BQ, D, 8, BQ), f32),
            vmem((KC_VPU // 8 * dh, 8, 128), f32),
            vmem((KC_VPU // 8 * dh, 8, 128), f32),
            vmem((KC // 16, 8, 128), u32),
            vmem((KC // 16, 8, 128), u32),
            vmem((5, D // 2, F // 2), bf16),
            vmem((5, F // 2, D // 2), bf16),
            pltpu.SemaphoreType.DMA((7,)),
        ],
        compiler_params=pltpu.CompilerParams(vmem_limit_bytes=96 * 2**20),
        name="fused_block",
    )(A_x, A_wqkv, A_wo, B_w1, B_b1, B_w2, B_b2)
```

```python
import functools
import math

import jax
import jax.numpy as jnp
from jax import lax
from jax.experimental import pallas as pl
from jax.experimental.pallas import tpu as pltpu

f32, bf16, u32 = jnp.float32, jnp.bfloat16, jnp.uint32

HEADS = 32
EPS = 1e-5
SUM_MIN, SUM_MAX = 2.0 ** -40, 2.0 ** 60
FINITE_MAX = 3.0e38

BQ = 512
TQ = BQ // 128
KC = 128
KC_VPU = 16
PV_LAG = 2
HEADS_PER_ITER = 4
D_GROUP = 4
X_PARTS = (384, 1024, 2048)
MLP_ROWS = 256
MLP_COLS = 384


def _layernorm(x):
    mu = jnp.mean(x, axis=-1, keepdims=True)
    xc = x - mu
    var = jnp.mean(xc * xc, axis=-1, keepdims=True)
    return xc * lax.rsqrt(var + EPS)


def _gelu(x):
    c = math.sqrt(2.0 / math.pi)
    u = x * (c + (c * 0.044715) * (x * x))
    hx = 0.5 * x
    return hx + hx * jnp.tanh(u)


def _dot(a, b):
    return jnp.dot(a, b, preferred_element_type=f32)


def _all_true(zero):
    return lax.broadcasted_iota(jnp.int32, (8, 128), 0) >= zero


def _strassen_weight_sums(w_ref, t_ref, row, n, keep, after):
    kh, nh = w_ref.shape[0] // 2, w_ref.shape[1] // 2
    top = w_ref[pl.ds(row, n), :].astype(f32)
    bot = w_ref[pl.ds(kh + row, n), :].astype(f32)
    b11, b12, b21, b22 = top[:, :nh], top[:, nh:], bot[:, :nh], bot[:, nh:]
    reps = (n // 8, nh // 128)
    b11 = jnp.where(jnp.tile(keep, reps), b11, jnp.tile(after, reps))
    b22 = jnp.where(jnp.tile(keep, reps), b22, jnp.tile(after, reps))
    for i, t in enumerate((b11 + b22, b12 - b22, b21 - b11, b11 + b12, b21 + b22)):
        t_ref[i, pl.ds(row, n), :] = t.astype(bf16)


def _strassen_rhs(w_ref, t_ref, rows, cols):
    kh, nh = w_ref.shape[0] // 2, w_ref.shape[1] // 2
    rows2 = slice(kh + rows.start, kh + rows.stop)
    cols2 = slice(nh + cols.start, nh + cols.stop)
    return [t_ref[0, rows, cols], w_ref[rows, cols], t_ref[1, rows, cols], t_ref[2, rows, cols],
            w_ref[rows2, cols2], t_ref[3, rows, cols], t_ref[4, rows, cols]]


def _strassen_lhs(a11, a12, a21, a22):
    return [t.astype(bf16) for t in (a11 + a22, a21 + a22, a11, a22, a11 + a12, a21 - a11, a12 - a22)]


def _strassen_result(m):
    return m[0] + m[3] - m[4] + m[6], m[2] + m[4], m[1] + m[3], m[0] - m[1] + m[2] + m[5]


def _kernel(x_hbm, wqkv_hbm, wo_hbm, w1_hbm, b1_hbm, w2_hbm, b2_hbm, out_hbm,
            x_buf, wq, wkv, wo, w1, b1, w2, b2, out_buf, ln_buf,
            k_buf, qt_buf, vt_buf, ot_buf, kf_buf, qv_buf, kb0, kb1, kh0, kh1, t1, t2, sems):
    S, D = x_buf.shape
    F = w1.shape[1]
    dh = D // HEADS
    heads_per_group = 128 // dh
    nq, nc = S // BQ, S // KC
    q_scale = dh ** -0.5 * math.log2(math.e)

    def copy(src, dst, sem):
        return pltpu.make_async_copy(src, dst, sems.at[sem])

    def out_copy(i):
        rows = pl.ds(pl.multiple_of(i * MLP_ROWS, MLP_ROWS), MLP_ROWS)
        return copy(out_buf.at[rows], out_hbm.at[0, rows], 4)

    wq_copy = copy(wqkv_hbm.at[:, pl.ds(0, D)], wq, 0)
    wkv_copy = copy(wqkv_hbm.at[:, pl.ds(D, 2 * D)], wkv, 1)
    w1_copy = copy(w1_hbm, w1, 2)
    mlp_copies = [copy(w2_hbm, w2, 3), copy(wo_hbm, wo, 3),
                  copy(b1_hbm, b1.at[pl.ds(0, F)], 3), copy(b2_hbm, b2.at[pl.ds(0, D)], 3)]
    x_copies = [copy(x_hbm.at[0, pl.ds(a, b - a)], x_buf.at[pl.ds(a, b - a)], 5 + n)
                for n, (a, b) in enumerate(zip((0,) + X_PARTS, X_PARTS))]
    for c in (x_copies[0], wq_copy, *x_copies[1:], wkv_copy):
        c.start()

    def norm_rows(r):
        ln = _layernorm(x_buf[pl.ds(r, 128), :].astype(f32)).astype(bf16)
        ln_buf[pl.ds(r, 128), :] = ln
        return ln

    def store_q(r, q):
        qt = pltpu.bitcast((q * q_scale).T.astype(bf16), u32)
        qt_buf[:, r // BQ, r % BQ // 128] = qt.reshape(HEADS, 8, 128)

    ln, qs = {}, {}
    normed = projected = stored = 0
    for x_copy, end in zip(x_copies, X_PARTS):
        x_copy.wait()
        if normed == 0:
            normed = 256
            for r in range(0, normed, 128):
                ln[r] = norm_rows(r)
            wq_copy.wait()
        left = 0 if end == S else 128
        for r in range(normed, end, 128):
            ln[r] = norm_rows(r)
        for r in range(projected, end - left, 128):
            qs[r] = _dot(ln[r], wq[...])
        for r in range(stored, end - 2 * left, 128):
            store_q(r, qs[r])
        normed, projected, stored = end, end - left, end - 2 * left
    for c in (w1_copy, *mlp_copies):
        c.start()
    wkv_copy.wait()
    w1_copy.wait()

    def project_kv(i, _):
        keep = _all_true(i // S)

        def replicate_q(h, d, after):
            q = jnp.where(keep, qt_buf[h, i], pltpu.bitcast(after, u32))
            q = jnp.concatenate([q[t] for t in range(TQ)], axis=1)
            q = pltpu.bitcast(q, bf16).astype(f32)
            rows = [jnp.broadcast_to(q[r:r + 1], (8, BQ)) for r in range(d, d + 4)]
            qv_buf[i, pl.ds(h * dh + d, 4)] = jnp.stack(rows)

        fill = [functools.partial(replicate_q, h, d) for h in range(HEADS) for d in range(0, dh, 4)]
        w1_rows = D // 2 // nq
        for n, r in enumerate(range(0, w1_rows, 16)):
            fill.insert(n * (len(fill) * 16 // w1_rows), functools.partial(
                _strassen_weight_sums, w1, t1, pl.multiple_of(i * w1_rows + r, 16), 16, keep))
        n_dots = TQ * (2 * D // 128)
        dots_done, fill_done = 0, 0

        def dot_and_fill(a, b):
            nonlocal dots_done, fill_done
            y = _dot(a, b)
            dots_done += 1
            last = min((dots_done + 1) * len(fill) // n_dots, len(fill))
            for n in range(fill_done, last):
                r = (n - fill_done) * (y.shape[0] // 8) // (last - fill_done) * 8
                fill[n](y[r:r + 8, :128])
            fill_done = last
            return y

        for t in range(TQ):
            blk = i * TQ + t
            a = ln_buf[pl.ds(pl.multiple_of(blk * 128, 128), 128), :]
            v = jnp.concatenate([dot_and_fill(a, wkv[:, D + c:D + c + 128]) for c in range(0, D, 128)], axis=1)
            k = jnp.concatenate([dot_and_fill(a, wkv[:, c:c + 128]) for c in range(0, D, 128)], axis=1)
            k = k.astype(bf16)
            vt_buf[:, i, t] = pltpu.bitcast(v.T.astype(bf16), u32).reshape(HEADS, 8, 128)
            k_packed = pltpu.bitcast(k, u32)
            for g in range(D // 128):
                k_buf[g, blk] = k_packed[:, g * 128:(g + 1) * 128]
                kf_buf[g, i, t] = k[:KC_VPU, g * 128:(g + 1) * 128].astype(f32)
        return None

    lax.fori_loop(0, nq, project_kv, None)

    k_heads, k_bcast = (kh0, kh1), (kb0, kb1)
    n_kh = (KC - KC_VPU) // 16
    n_kb = KC_VPU // 8 * dh

    def head_shift(h):
        return (128 - (h % heads_per_group) * dh) % 128

    def stage_keys(h, j, part, parts):
        g, shift = h // heads_per_group, head_shift(h)
        lo, hi = part * n_kh // parts, (part + 1) * n_kh // parts
        k = pltpu.roll(k_buf[g, j, KC_VPU // 2 + lo * 8:KC_VPU // 2 + hi * 8], shift, 1)
        k_heads[j % 2][lo:hi] = k.reshape(hi - lo, 8, 128)
        lo, hi = part * n_kb // parts, (part + 1) * n_kb // parts
        r0, r1 = lo // dh, (hi - 1) // dh + 1
        k = pltpu.roll(kf_buf[g, j // TQ, j % TQ, r0 * 8:r1 * 8, :], shift, 1)
        cols = [k[(e // dh - r0) * 8:(e // dh - r0 + 1) * 8, e % dh:e % dh + 1] for e in range(lo, hi)]
        k_bcast[j % 2][lo:hi] = jnp.stack([jnp.broadcast_to(c, (8, 128)) for c in cols])

    def attend_unshifted(it, unsafe):
        zero = it // HEADS
        keep = _all_true(zero)
        o_zero = jnp.full((dh, BQ), zero, jnp.int32).astype(f32)
        per_head = nc * nq
        steps = HEADS_PER_ITER * per_head
        rows_mxu = 2 * n_kh
        groups = n_kb // D_GROUP
        sums, outs, probs, scores = {}, {}, {}, []
        for n in range(steps + PV_LAG):
            z = zero * (n + 1)
            if n < steps:
                u, (j, qb) = n // per_head, divmod(n % per_head, nq)
                h = it * HEADS_PER_ITER + u
                q = qt_buf[h, qb + z]
                q = jnp.concatenate([q[t] for t in range(TQ)], axis=1)
                k = k_heads[j % 2][pl.ds(z, n_kh)].reshape(n_kh * 8, 128)
                scores.append(_dot(pltpu.bitcast(k, bf16)[:, :dh], pltpu.bitcast(q, bf16)))
            if n >= PV_LAG:
                uo, (jo, qo) = (n - PV_LAG) // per_head, divmod((n - PV_LAG) % per_head, nq)
                v = vt_buf[it * HEADS_PER_ITER + uo, jo // TQ + z, jo % TQ]
                pv = _dot(pltpu.bitcast(v, bf16), probs.pop(n - PV_LAG))
                outs[qo] = (o_zero if jo == 0 else outs[qo]) + pv
            if n < steps:
                p_mxu = jnp.exp2(scores[n])
                if j + 1 < nc:
                    stage_keys(h, j + 1, qb, nq)
                else:
                    stage_keys(jnp.minimum(h + 1, HEADS - 1), 0, qb, nq)
                p_vpu = []
                k_cols = k_bcast[j % 2][pl.ds(z, n_kb)]
                for r in range(KC_VPU // 8):
                    s = None
                    q_rows = qv_buf[qb, pl.ds(h * dh + zero * (4 * n + r + 1), dh)]
                    for d in range(0, dh, D_GROUP):
                        qv = q_rows[d:d + D_GROUP]
                        kv = k_cols[r * dh + d:r * dh + d + D_GROUP]
                        pos = (n - 1) * rows_mxu + (r * dh + d) // D_GROUP * rows_mxu // groups + 3
                        if pos >= 0:
                            step, row = divmod(pos, rows_mxu)
                            first = jnp.where(keep, kv[0], scores[step][row * 8:(row + 1) * 8, :128])
                            kv = jnp.concatenate([first[None], kv[1:]], axis=0)
                        prod = jnp.concatenate([kv] * TQ, axis=2) * qv
                        for c in range(D_GROUP):
                            s = prod[c] if s is None else s + prod[c]
                    p_vpu.append(jnp.exp2(s))
                total = sums[u, qb] if j else None
                rows = [p_mxu[r * 8:(r + 1) * 8] for r in range(rows_mxu)]
                for p in rows[:10] + p_vpu + rows[10:]:
                    total = p if total is None else total + p
                sums[u, qb] = total
                probs[n] = jnp.concatenate(p_vpu + [p_mxu], axis=0).astype(bf16)
            if n >= PV_LAG and jo == nc - 1:
                total = jnp.sum(sums[uo, qo], axis=0, keepdims=True)
                o = outs[qo] * (1.0 / total)
                pair, odd = it * (HEADS_PER_ITER // 2) + uo // 2, uo % 2
                for t in range(TQ):
                    ot_buf[qo * TQ + t, pair, odd * dh:(odd + 1) * dh, :] = o[:, t * 128:(t + 1) * 128]
                safe = ((total >= SUM_MIN) & (total <= SUM_MAX)
                        & (jnp.abs(o[:8]) + jnp.abs(o[8:]) <= FINITE_MAX))
                unsafe = jnp.where(safe, unsafe, 1.0)
        w2_rows = F // 2 // (HEADS // HEADS_PER_ITER)
        for r in range(0, w2_rows, 16):
            _strassen_weight_sums(w2, t2, pl.multiple_of(it * w2_rows + r, 16), 16, keep, scores[-1][56:64, :128])
        return unsafe

    def attend_with_max(n, _):
        h, qb = n // nq, n % nq
        q = pltpu.bitcast(jnp.concatenate([qt_buf[h, qb, t] for t in range(TQ)], axis=1), bf16)
        rows = BQ // 8

        def row_max(c, m):
            k = k_buf[h // heads_per_group, pl.ds(c * TQ, TQ)].reshape(BQ // 2, 128)
            k = pltpu.bitcast(pltpu.roll(k, head_shift(h), 1), bf16)
            s = _dot(k[:, :dh], q).reshape(rows, 8, BQ)
            qv_buf[0, pl.ds(c * rows, rows)] = s
            return jnp.maximum(m, jnp.max(s, axis=0))

        m = lax.fori_loop(0, S // BQ, row_max, jnp.full((8, BQ), -jnp.inf, f32))
        m = jnp.max(m, axis=0, keepdims=True)

        def accumulate(c, acc):
            p = jnp.exp2(qv_buf[0, pl.ds(c * rows, rows)] - m)
            v = jnp.concatenate([vt_buf[h, c, t] for t in range(TQ)], axis=1)
            return (acc[0] + jnp.sum(p, axis=0),
                    acc[1] + _dot(pltpu.bitcast(v, bf16), p.reshape(BQ, BQ).astype(bf16)))

        total, o = lax.fori_loop(0, S // BQ, accumulate, (jnp.zeros((8, BQ), f32), jnp.zeros((dh, BQ), f32)))
        o = o * (1.0 / jnp.sum(total, axis=0, keepdims=True))
        for t in range(TQ):
            ot_buf[qb * TQ + t, h // 2, pl.ds(pl.multiple_of(h % 2 * dh, dh), dh), :] = o[:, t * 128:(t + 1) * 128]
        return None

    for c in mlp_copies:
        c.wait()
    stage_keys(0, 0, 0, 1)
    unsafe = lax.fori_loop(0, HEADS // HEADS_PER_ITER, attend_unshifted, jnp.zeros((8, BQ), f32))

    @pl.when(jnp.max(unsafe) > 0.0)
    def _():
        lax.fori_loop(0, HEADS * nq, attend_with_max, None)

    def mlp(i, _):
        bias1 = b1[pl.ds(0, F)].astype(f32).reshape(1, F)
        bias2 = b2[pl.ds(0, D)].astype(f32).reshape(1, D)
        starts = [pl.multiple_of(i * BQ + r, MLP_ROWS) for r in range(0, BQ, MLP_ROWS)]
        hs, lns = [], []
        for r in starts:
            o = [ot_buf[r // 128 + t].reshape(D, 128).T for t in range(MLP_ROWS // 128)]
            o = jnp.concatenate(o, axis=0)
            h = x_buf[pl.ds(r, MLP_ROWS), :].astype(f32) + _dot(o.astype(bf16), wo[...])
            hs.append(h)
            lns.append(_layernorm(h))
        mh, kh, fh = MLP_ROWS // 2, D // 2, F // 2
        chunks = [slice(c, min(c + MLP_COLS, fh)) for c in range(0, fh, MLP_COLS)]
        for n, (r, h, a) in enumerate(zip(starts, hs, lns)):
            lhs = _strassen_lhs(a[:mh, :kh], a[:mh, kh:], a[mh:, :kh], a[mh:, kh:])
            acc = [None] * 7
            prev = None
            for c in range(len(chunks) + 1):
                cur = None
                if c < len(chunks):
                    left = chunks[c]
                    right = slice(fh + left.start, fh + left.stop)
                    c11, c12, c21, c22 = _strassen_result(
                        [_dot(y, w) for y, w in zip(lhs, _strassen_rhs(w1, t1, slice(0, kh), left))])
                    cur = _strassen_lhs(_gelu(c11 + bias1[:, left]), _gelu(c12 + bias1[:, right]),
                                        _gelu(c21 + bias1[:, left]), _gelu(c22 + bias1[:, right]))
                if prev is not None:
                    for b, (y, w) in enumerate(zip(prev, _strassen_rhs(w2, t2, chunks[c - 1], slice(0, kh)))):
                        acc[b] = _dot(y, w) if acc[b] is None else acc[b] + _dot(y, w)
                prev = cur
            c11, c12, c21, c22 = _strassen_result(acc)
            y = jnp.concatenate([jnp.concatenate([c11, c12], axis=1), jnp.concatenate([c21, c22], axis=1)], axis=0)
            out_buf[pl.ds(r, MLP_ROWS), :] = (h + bias2 + y).astype(bf16)
            out_copy(i * len(starts) + n).start()
        return None

    lax.fori_loop(0, nq, mlp, None)
    for i in range(S // MLP_ROWS):
        out_copy(i).wait()


@jax.jit
def pallas_sequential_preLN__softmax_full_mha__dense_activation_gelu__prompt_kernel(
    A_x: jax.Array,
    A_wqkv: jax.Array,
    A_wo: jax.Array,
    B_x: jax.Array,
    B_w1: jax.Array,
    B_b1: jax.Array,
    B_w2: jax.Array,
    B_b2: jax.Array,
):
    del B_x
    batch, S, D = A_x.shape
    F = B_w1.shape[1]
    assert (batch, S, D, F) == (1, 2048, 512, 1792)
    dh = D // HEADS
    vmem = pltpu.VMEM
    in_hbm = pl.BlockSpec(memory_space=pl.ANY)
    return pl.pallas_call(
        _kernel,
        in_specs=[in_hbm] * 7,
        out_specs=in_hbm,
        out_shape=jax.ShapeDtypeStruct(A_x.shape, A_x.dtype),
        scratch_shapes=[
            vmem((S, D), bf16),
            vmem((D, D), bf16),
            vmem((D, 2 * D), bf16),
            vmem((D, D), bf16),
            vmem((D, F), bf16),
            vmem((8192,), bf16),
            vmem((F, D), bf16),
            vmem((8192,), bf16),
            vmem((S, D), bf16),
            vmem((S, D), bf16),
            vmem((D // 128, S // KC, KC // 2, 128), u32),
            vmem((HEADS, S // BQ, TQ, dh // 2, 128), u32),
            vmem((HEADS, S // BQ, TQ, dh // 2, 128), u32),
            vmem((S // 128, HEADS // 2, 2 * dh, 128), f32),
            vmem((D // 128, S // BQ, TQ, KC_VPU, 128), f32),
            vmem((S // BQ, D, 8, BQ), f32),
            vmem((KC_VPU // 8 * dh, 8, 128), f32),
            vmem((KC_VPU // 8 * dh, 8, 128), f32),
            vmem((KC // 16, 8, 128), u32),
            vmem((KC // 16, 8, 128), u32),
            vmem((5, D // 2, F // 2), bf16),
            vmem((5, F // 2, D // 2), bf16),
            pltpu.SemaphoreType.DMA((5 + len(X_PARTS),)),
        ],
        compiler_params=pltpu.CompilerParams(vmem_limit_bytes=96 * 2**20),
        name="fused_block",
    )(A_x, A_wqkv, A_wo, B_w1, B_b1, B_w2, B_b2)
```
